```python
import jax
import jax.numpy as jnp

def _softmax(x, axis=-1):
    return jax.nn.softmax(x, axis=axis)

def _gelu(x):
    return jax.nn.gelu(x, approximate=True)

def _silu(x):
    return jax.nn.silu(x)

def _sigmoid(x):
    return jax.nn.sigmoid(x)

def _layernorm(x, axis=-1, eps=1e-05):
    m = jnp.mean(x, axis=axis, keepdims=True)
    v = jnp.var(x, axis=axis, keepdims=True)
    return (x - m) / jnp.sqrt(v + eps)

def _scatter_add(tgt, idx, src, axis=0):
    return tgt.at[idx].add(src)

def _segment_sum(src, seg, n):
    return jax.ops.segment_sum(src, seg, n)

class _Rng:

    def __init__(self, key):
        self._k = key

    def _next(self):
        self._k, sub = jax.random.split(self._k)
        return sub

    def normal(self, shape):
        return jax.random.normal(self._next(), shape, dtype=jnp.bfloat16)

    def randint(self, lo, hi, shape):
        return jax.random.randint(self._next(), shape, lo, hi, dtype=jnp.int32)

    def uniform(self, shape, lo=0.0, hi=1.0):
        return jax.random.uniform(self._next(), shape, jnp.bfloat16, lo, hi)

    def permutation(self, n):
        return jax.random.permutation(self._next(), n)
kernel_name = 'adaLN_cond__compressed_kv_cla__moe_arch_mod__prompt'

def setup_inputs():
    _rng = _Rng(jax.random.key(int.from_bytes(__import__("os").urandom(4), "little")))
    _w = lambda a: (lambda t: t.astype(jnp.bfloat16) if jnp.issubdtype(t.dtype, jnp.floating) else t)(jnp.asarray(a))

    def _A_setup():
        B, H, Sq, Sk, D, M = (1, 32, 2048, 2048, 128, 640)
        Dc = 4 * D
        return {'x': _w((lambda *s: _rng.normal(s) * 0.05)(B, Sq, M)), 'c_kv': _w((lambda *s: _rng.normal(s) * 0.05)(B, Sk, Dc)), 'w_q': _w((lambda *s: _rng.normal(s) * 0.05)(M, H, D) * M ** (-0.5)), 'w_uk': _w((lambda *s: _rng.normal(s) * 0.05)(Dc, H, D) * Dc ** (-0.5)), 'w_uv': _w((lambda *s: _rng.normal(s) * 0.05)(Dc, H, D) * Dc ** (-0.5)), 'w_o': _w((lambda *s: _rng.normal(s) * 0.05)(H, D, M) * (H * D) ** (-0.5))}
    _A_in = _A_setup()

    def _B_setup():
        B, S, D, F, C = (1, 2048, 640, 1728, 8)
        return {'x': _w((lambda *s: _rng.normal(s) * 0.05)(B, S, D)), 'w_r': _w((lambda *s: _rng.normal(s) * 0.05)(D)), 'w_gate': _w((lambda *s: _rng.normal(s) * 0.05)(D, F)), 'w_up': _w((lambda *s: _rng.normal(s) * 0.05)(D, F)), 'w_down': _w((lambda *s: _rng.normal(s) * 0.05)(F, D))}
    _B_in = _B_setup()
    return {'A_x': _A_in['x'], 'A_c_kv': _A_in['c_kv'], 'A_w_q': _A_in['w_q'], 'A_w_uk': _A_in['w_uk'], 'A_w_uv': _A_in['w_uv'], 'A_w_o': _A_in['w_o'], 'B_x': _B_in['x'], 'B_w_r': _B_in['w_r'], 'B_w_gate': _B_in['w_gate'], 'B_w_up': _B_in['w_up'], 'B_w_down': _B_in['w_down'], 'c': _w((lambda *s: _rng.normal(s) * 0.05)(1, 640)), 'w_mod': _w((lambda *s: _rng.normal(s) * 0.05)(640, 6 * 640) * 640 ** (-0.5))}

def reference(A_x, A_c_kv, A_w_q, A_w_uk, A_w_uv, A_w_o, B_x, B_w_r, B_w_gate, B_w_up, B_w_down, c, w_mod):

    def _A_ref(x, c_kv, w_q, w_uk, w_uv, w_o):
        B, Sq, M = (x.shape[0], x.shape[1], x.shape[2])
        Sk = c_kv.shape[1]
        H, D = (w_q.shape[1], w_q.shape[2])
        q = jnp.einsum('bqm,mhd->bhqd', x, w_q)
        k = jnp.einsum('bkc,chd->bhkd', c_kv, w_uk)
        v = jnp.einsum('bkc,chd->bhkd', c_kv, w_uv)
        scores = jnp.einsum('bhqd,bhkd->bhqk', q, k) * D ** (-0.5)
        off = Sk - Sq
        qi = jnp.arange(Sq)[:, None]
        kj = jnp.arange(Sk)[None, :]
        cmask = kj <= qi + off
        scores = jnp.where(cmask[None, None], scores, -1000000000.0)
        p = _softmax(scores, axis=-1)
        ctx = jnp.einsum('bhqk,bhkd->bhqd', p, v)
        return jnp.einsum('bhqd,hdm->bqm', ctx, w_o)

    def _B_ref(x, w_r, w_gate, w_up, w_down):
        B, S, D = x.shape
        C = 8
        r = x @ w_r
        idx = jnp.argsort(-r, axis=-1)[:, :C]
        idx_e = jnp.repeat(idx.reshape(B, C, 1), D, axis=2)
        x_sel = jnp.take_along_axis(x, idx_e, axis=1)
        g = _silu(x_sel @ w_gate)
        u = x_sel @ w_up
        y = g * u @ w_down
        r_sel = _sigmoid(jnp.take_along_axis(r, idx, axis=1))
        y = y * r_sel.reshape(B, C, 1)
        b_off = (jnp.arange(B) * S).reshape(B, 1)
        flat_idx = (idx + b_off).reshape(B * C)
        zero = (x * 0.0).reshape(B * S, D)
        upd = _scatter_add(zero, flat_idx, y.reshape(B * C, D), axis=0)
        return x + upd.reshape(B, S, D)
    x = A_x
    mod = (_silu(c) @ w_mod).reshape(c.shape[0], 6, 1, -1)
    sa, ca, ga, sb, cb, gb = (mod[:, 0].copy(), mod[:, 1].copy(), mod[:, 2].copy(), mod[:, 3].copy(), mod[:, 4].copy(), mod[:, 5].copy())
    h = _layernorm(x, axis=-1) * (1 + ca) + sa
    x = x + ga * _A_ref(h, A_c_kv, A_w_q, A_w_uk, A_w_uv, A_w_o)
    h = _layernorm(x, axis=-1) * (1 + cb) + sb
    x = x + gb * _B_ref(h, B_w_r, B_w_gate, B_w_up, B_w_down)
    return x
```

```python
import math

import jax
import jax.numpy as jnp
import ml_dtypes
import numpy as np
from jax import lax
import jax.experimental.pallas as pl
import jax.experimental.pallas.tpu as pltpu

F32 = jnp.float32
BF16 = jnp.bfloat16
T = 128
TOPK = 8
HG = 8
NT = (((1,), (1,)), ((), ()))
LOG2E = math.log2(math.e)
EPS = float(np.float32(ml_dtypes.bfloat16(1e-05)))
MASK = float(np.float32(ml_dtypes.bfloat16(-1000000000.0))) * LOG2E
KEY_BASE = 0x20000000


def _rb(v):
    return v.astype(BF16).astype(F32)


def _sigmoid(z):
    return _rb(1.0 / _rb(1.0 + _rb(jnp.exp(-z))))


def _ln_mod(x, scale1, shift):
    inv_n = 1.0 / x.shape[-1]
    mean = jnp.sum(x, axis=-1, keepdims=True) * inv_n
    cen = x - mean
    var = _rb(jnp.sum(cen * cen, axis=-1, keepdims=True) * inv_n)
    rstd = 1.0 / _rb(jnp.sqrt(_rb(var + EPS)))
    n = _rb(_rb(x - _rb(mean)) * rstd)
    return _rb(_rb(n * scale1) + shift)


def _head_jobs(nb, look=1, olag=4, qc=4):
    seq = list(range(nb))[::-1]
    jobs, qdone = [], set()

    def need_q(i):
        if i // qc not in qdone:
            qdone.add(i // qc)
            jobs.append(("q", i // qc * qc, qc))

    need_q(seq[0])
    jobs += [("v", 0, nb // 2), ("v", nb // 2, nb // 2)]
    for t in range(nb + look + olag):
        if t + 2 < nb:
            need_q(seq[t + 2])
        if t < nb:
            need_q(seq[t])
            jobs.append(("p1", seq[t]))
        if 0 <= t - look < nb:
            jobs.append(("p2", seq[t - look]))
        if 0 <= t - look - olag < nb:
            jobs.append(("o", seq[t - look - olag]))
    return jobs


def _kernel(x_hbm, ckv_hbm, wq_hbm, wuk_hbm, wuv_hbm, wo_hbm, wr_hbm, wg_hbm,
            wu_hbm, wd_hbm, c_hbm, wmod_hbm, out_hbm,
            x_v, ckv_v, wq_raw, wuk_raw, wuv_raw, wo_v, wr_v, wg_v, wu_v, wd_v,
            c_v, wmod_v, wq_s, wuk_s, wuv_s, k_s, v_s, h_s, acc_s, h2_s, out_s,
            mod_s, sems, osems):
    S, M = x_v.shape
    H, _, D = k_s.shape
    nb = S // T
    ng = H // HG
    qscale = D ** -0.5 * LOG2E
    r0 = S // 4

    names = ["ckv0", "ckv1", "x", "wq", "wuv", "wo", "wr", "wg", "wu", "wd", "c",
             "wmod"] + ["wuk%d" % g for g in range(ng)]
    pairs = {
        "ckv0": (ckv_hbm.at[pl.ds(0, r0)], ckv_v.at[pl.ds(0, r0)]),
        "ckv1": (ckv_hbm.at[pl.ds(r0, S - r0)], ckv_v.at[pl.ds(r0, S - r0)]),
        "x": (x_hbm, x_v), "wq": (wq_hbm, wq_raw), "wuv": (wuv_hbm, wuv_raw),
        "wo": (wo_hbm, wo_v), "wr": (wr_hbm, wr_v), "wg": (wg_hbm, wg_v),
        "wu": (wu_hbm, wu_v), "wd": (wd_hbm, wd_v), "c": (c_hbm, c_v),
        "wmod": (wmod_hbm, wmod_v),
    }
    for g in range(ng):
        pairs["wuk%d" % g] = (wuk_hbm.at[:, pl.ds(g * HG, HG), :], wuk_raw.at[g])
    cp = {n: pltpu.make_async_copy(*pairs[n], sems.at[i]) for i, n in enumerate(names)}

    def start(*ns):
        for n in ns:
            cp[n].start()

    def wait(*ns):
        for n in ns:
            cp[n].wait()

    def split_heads(raw, dst, h0, lo, n):
        nh = raw.shape[1]
        w = raw[lo:lo + n].reshape(n, nh * D)
        for j in range(nh):
            dst[h0 + j, lo:lo + n, :] = w[:, j * D:(j + 1) * D]

    def split_jobs(raw, dst, h0, n):
        return [lambda lo=lo: split_heads(raw, dst, h0, lo, n)
                for lo in range(0, raw.shape[0], n)]

    def kproj(h, lo, n):
        k_s[h, lo:lo + n, :] = jnp.dot(
            ckv_v[lo:lo + n, :], wuk_s[h], preferred_element_type=F32).astype(BF16)

    def kproj_group(g, lo, n, side):
        for j in range(HG):
            kproj(g * HG + j, lo, n)
            for job in side[len(side) * j // HG:len(side) * (j + 1) // HG]:
                job()

    def zero_acc(i):
        acc_s[i * T:(i + 1) * T, :] = jnp.zeros((T, M), F32)

    col = {}

    def silu_col():
        c = c_v[...].astype(F32)
        col["c"] = jnp.broadcast_to(_rb(c * _sigmoid(c)), (T, M)).T

    def mod_tile(j):
        p, o = divmod(j * T, M)
        w = wmod_v[:, j * T:(j + 1) * T].astype(F32)
        m = _rb(jnp.sum(w * col["c"], axis=0, keepdims=True))
        if p in (1, 4):
            m = _rb(1.0 + m)
        mod_s[p:p + 1, o:o + T] = m

    def ln1(i):
        x = x_v[i * T:(i + 1) * T, :].astype(F32)
        h_s[i * T:(i + 1) * T, :] = _ln_mod(x, mod_s[1:2, :], mod_s[0:1, :]).astype(BF16)

    start("wuk0", "ckv0")
    start("ckv1", "wuk1")
    wait("wuk0")
    for job in split_jobs(wuk_raw.at[0], wuk_s, 0, 64):
        job()
    wait("ckv0")
    start("wuk2", "wuk3", "c", "wmod")
    kproj_group(0, 0, r0, [lambda i=i: zero_acc(i) for i in range(nb)])
    wait("ckv1", "wuk1")
    start("x", "wq")
    kproj_group(0, r0, S - r0, split_jobs(wuk_raw.at[1], wuk_s, HG, 64))
    wait("wuk2", "wuk3", "c", "wmod")
    start("wuv", "wo")
    kproj_group(1, 0, S,
                split_jobs(wuk_raw.at[2], wuk_s, 2 * HG, 64)
                + [silu_col] + [lambda j=j: mod_tile(j) for j in range(6 * M // T)])
    wait("x", "wq")
    start("wr", "wg", "wu", "wd")
    kproj_group(2, 0, S,
                split_jobs(wuk_raw.at[3], wuk_s, 3 * HG, 64)
                + [lambda i=i: ln1(i) for i in range(nb)])
    wait("wuv", "wo")
    kproj_group(3, 0, S,
                split_jobs(wq_raw, wq_s, 0, 16) + split_jobs(wuv_raw, wuv_s, 0, 16))

    def head(h, finish):
        tri = (lax.broadcasted_iota(jnp.int32, (T, T), 1)
               <= lax.broadcasted_iota(jnp.int32, (T, T), 0))
        q, st, ctx = {}, {}, {}
        for job in _head_jobs(nb):
            kind, i = job[0], job[1]
            if kind == "q":
                n = job[2]
                r = jnp.dot(h_s[i * T:(i + n) * T, :], wq_s[h], preferred_element_type=F32)
                for a in range(n):
                    q[i + a] = (r[a * T:(a + 1) * T] * qscale).astype(BF16)
            elif kind == "v":
                n = job[2]
                v_s[i * T:(i + n) * T, :] = jnp.dot(
                    ckv_v[i * T:(i + n) * T, :], wuv_s[h],
                    preferred_element_type=F32).astype(BF16)
            elif kind == "p1":
                s = lax.dot_general(q.pop(i), k_s[h, :(i + 1) * T, :], NT,
                                    preferred_element_type=F32)
                tiles = [s[:, j * T:(j + 1) * T] for j in range(i + 1)]
                tiles[-1] = jnp.where(tri, tiles[-1], MASK)
                m = tiles[0]
                for t in tiles[1:]:
                    m = jnp.maximum(m, t)
                st[i] = (jnp.max(m, axis=1, keepdims=True), tiles)
            elif kind == "p2":
                m, tiles = st.pop(i)
                ps = [jnp.exp2(t - m) for t in tiles]
                l = ps[0]
                for p in ps[1:]:
                    l = l + p
                l = jnp.sum(l, axis=1, keepdims=True)
                o = jnp.dot(jnp.concatenate(ps, axis=1).astype(BF16),
                            v_s[:(i + 1) * T, :], preferred_element_type=F32)
                r = pltpu.reciprocal(l, approx=True)
                r = r * (2.0 - l * r)
                ctx[i] = (o * r).astype(BF16)
            else:
                finish(i, acc_s[i * T:(i + 1) * T, :] + jnp.dot(
                    ctx.pop(i), wo_v[h], preferred_element_type=F32))

    def accumulate(i, attn):
        acc_s[i * T:(i + 1) * T, :] = attn

    def loop_body(h, carry):
        head(h, accumulate)
        return carry

    lax.fori_loop(0, H - 1, loop_body, 0)

    wait("wr", "wg", "wu", "wd")
    w_r = wr_v[...].astype(F32).reshape(1, M)
    lane = lax.broadcasted_iota(jnp.int32, (8, T), 1)
    per = T // 8
    nkey = S // (8 * T)
    scores = [jnp.zeros((8, T), F32) for _ in range(nkey)]
    nout = osems.shape[0] - TOPK
    ot = nb // nout
    out_cp = [pltpu.make_async_copy(out_s.at[pl.ds(j * ot * T, ot * T)],
                                    out_hbm.at[pl.ds(j * ot * T, ot * T)], osems.at[j])
              for j in range(nout)]
    todo = [ot] * nout

    def finalize(i, attn):
        rows = slice(i * T, (i + 1) * T)
        x1 = _rb(x_v[rows, :].astype(F32) + _rb(mod_s[2:3, :] * _rb(attn)))
        h2 = _ln_mod(x1, mod_s[4:5, :], mod_s[3:4, :])
        acc_s[rows, :] = x1
        h2_s[rows, :] = h2
        out_s[rows, :] = (x1 + _rb(mod_s[5:6, :] * (h2 + h2 * 0.0))).astype(BF16)
        r = jnp.sum(h2 * w_r, axis=1, keepdims=True)
        b, o = divmod(i * per, T)
        for j in range(per):
            scores[b] = jnp.where(lane == o + j, r[8 * j:8 * j + 8], scores[b])
        todo[i // ot] -= 1
        if todo[i // ot] == 0:
            out_cp[i // ot].start()

    head(H - 1, finalize)

    sub = lax.broadcasted_iota(jnp.int32, (8, T), 0)
    ibits = (S - 1).bit_length()
    keys = []
    for b in range(nkey):
        r = _rb(scores[b])
        u = lax.shift_right_logical(lax.bitcast_convert_type(r, jnp.int32), 16)
        u = jnp.where(u >= 0x8000, 0xFFFF - u, u + 0x8000)
        u = jnp.where(r == 0.0, 0x8000, u)
        u = jnp.where(r != r, 0, u)
        tok = b * 8 * T + 8 * lane + sub
        keys.append(lax.bitcast_convert_type(
            KEY_BASE + (u << ibits) + ((1 << ibits) - 1 - tok), F32))
    best = jnp.zeros((8, T), F32)
    for k in range(TOPK):
        m = keys[0]
        for kk in keys[1:]:
            m = jnp.maximum(m, kk)
        m = jnp.max(jnp.max(m, axis=1, keepdims=True), axis=0, keepdims=True)
        best = jnp.where(sub == k, m, best)
        keys = [jnp.where(kk == m, 0.0, kk) for kk in keys]
    bi = lax.bitcast_convert_type(best, jnp.int32) - KEY_BASE
    u = bi >> ibits
    u = jnp.where(u >= 0x8000, u - 0x8000, 0xFFFF - u)
    r_sel = lax.bitcast_convert_type(u << 16, F32)[:, 0:1]
    tok = (1 << ibits) - 1 - (bi & ((1 << ibits) - 1))
    idx = [jnp.clip(tok[k, 0], 0, S - 1) for k in range(TOPK)]

    hs = jnp.concatenate([h2_s[pl.ds(i, 1), :] for i in idx], axis=0)
    xs = jnp.concatenate([acc_s[pl.ds(i, 1), :] for i in idx], axis=0)
    hb = hs.astype(BF16)
    g = _rb(lax.dot_general(hb, wg_v[...], NT, preferred_element_type=F32))
    up = _rb(lax.dot_general(hb, wu_v[...], NT, preferred_element_type=F32))
    a = (_rb(g * _sigmoid(g)) * up).astype(BF16)
    y = _rb(jnp.dot(a, wd_v[...], preferred_element_type=F32))
    y = _rb(y * _sigmoid(r_sel))
    new = _rb(xs + _rb(mod_s[5:6, :] * _rb(hs + (hs * 0.0 + y))))

    for c_ in out_cp:
        c_.wait()
    row16 = lax.broadcasted_iota(jnp.int32, (16, M), 0)
    base = [pl.multiple_of((i // 16) * 16, 16) for i in idx]
    for k in range(TOPK):
        old = out_s[pl.ds(base[k], 16), :].astype(F32)
        out_s[pl.ds(base[k], 16), :] = jnp.where(
            row16 == idx[k] - base[k], new[k:k + 1, :], old).astype(BF16)
    first = []
    for k in range(TOPK):
        f = True
        for j in range(k):
            f = jnp.logical_and(f, base[j] != base[k])
        first.append(f)
    patch = [pltpu.make_async_copy(out_s.at[pl.ds(base[k], 16)],
                                   out_hbm.at[pl.ds(base[k], 16)], osems.at[nout + k])
             for k in range(TOPK)]
    for k in range(TOPK):
        pl.when(first[k])(patch[k].start)
    for k in range(TOPK):
        pl.when(first[k])(patch[k].wait)


@jax.jit
def pallas_adaLN_cond__compressed_kv_cla__moe_arch_mod__prompt_kernel(
    A_x: jax.Array,
    A_c_kv: jax.Array,
    A_w_q: jax.Array,
    A_w_uk: jax.Array,
    A_w_uv: jax.Array,
    A_w_o: jax.Array,
    B_x: jax.Array,
    B_w_r: jax.Array,
    B_w_gate: jax.Array,
    B_w_up: jax.Array,
    B_w_down: jax.Array,
    c: jax.Array,
    w_mod: jax.Array,
):
    del B_x
    B, S, M = A_x.shape
    C = A_c_kv.shape[2]
    _, H, D = A_w_q.shape
    F = B_w_gate.shape[1]
    assert B == 1 and A_c_kv.shape[1] == S and D == T and H == 4 * HG
    vm = pltpu.VMEM
    out = pl.pallas_call(
        _kernel,
        out_shape=jax.ShapeDtypeStruct((S, M), A_x.dtype),
        in_specs=[pl.BlockSpec(memory_space=pltpu.HBM)] * 12,
        out_specs=pl.BlockSpec(memory_space=pltpu.HBM),
        scratch_shapes=[
            vm((S, M), BF16), vm((S, C), BF16), vm((M, H, D), BF16),
            vm((H // HG, C, HG, D), BF16), vm((C, H, D), BF16), vm((H, D, M), BF16),
            vm((M,), BF16), vm((F, M), BF16), vm((F, M), BF16), vm((F, M), BF16),
            vm((1, M), BF16), vm((M, 6 * M), BF16),
            vm((H, M, D), BF16), vm((H, C, D), BF16), vm((H, C, D), BF16),
            vm((H, S, D), BF16), vm((S, D), BF16), vm((S, M), BF16),
            vm((S, M), F32), vm((S, M), F32), vm((S, M), BF16), vm((8, M), F32),
            pltpu.SemaphoreType.DMA((12 + H // HG,)),
            pltpu.SemaphoreType.DMA((4 + TOPK,)),
        ],
        compiler_params=pltpu.CompilerParams(vmem_limit_bytes=120 * 2 ** 20),
        name="adaln_cla_moe",
    )(A_x.reshape(S, M), A_c_kv.reshape(S, C), A_w_q, A_w_uk, A_w_uv, A_w_o,
      B_w_r, B_w_gate.T, B_w_up.T, B_w_down, c, w_mod)
    return out.reshape(B, S, M)
```

```python
import math

import jax
import jax.numpy as jnp
import ml_dtypes
import numpy as np
from jax import lax
import jax.experimental.pallas as pl
import jax.experimental.pallas.tpu as pltpu

F32 = jnp.float32
BF16 = jnp.bfloat16
U32 = jnp.uint32
T = 128
TOPK = 8
NOUT = 4
NT = (((1,), (1,)), ((), ()))
LOG2E = math.log2(math.e)
EPS = float(np.float32(ml_dtypes.bfloat16(1e-05)))
MASK = float(np.float32(ml_dtypes.bfloat16(-1000000000.0))) * LOG2E
KEY_BASE = 0x20000000


def _rb(v):
    return v.astype(BF16).astype(F32)


def _sigmoid(z):
    return _rb(1.0 / _rb(1.0 + _rb(jnp.exp(-z))))


def _recip(v):
    r = pltpu.reciprocal(v, approx=True)
    return r * (2.0 - v * r)


def _moments(x):
    inv_n = 1.0 / x.shape[-1]
    mean = jnp.sum(x, axis=-1, keepdims=True) * inv_n
    cen = x - mean
    return mean, cen, jnp.sum(cen * cen, axis=-1, keepdims=True) * inv_n


def _unzip(u):
    lo = lax.bitcast_convert_type(u << 16, F32)
    hi = lax.bitcast_convert_type(u & np.uint32(0xFFFF0000), F32)
    return jnp.concatenate([lo, hi], axis=1).astype(BF16)


def _ld(ref, lead, lo, n):
    return pltpu.bitcast(ref[lead + (pl.ds(lo // 2, n // 2),)], BF16)


def _st(ref, lead, lo, val):
    ref[lead + (pl.ds(lo // 2, val.shape[0] // 2),)] = pltpu.bitcast(val.astype(BF16), U32)


def _pair_jobs(nb, look, qlead, slag):
    tiles = []
    for a in range(nb // 2):
        tiles += [nb - 1 - a, a]
    units = [(e, i) for i in tiles for e in (0, 1)]
    n = len(units)
    jobs, qdone = [], set()

    def need_q(i):
        if i not in qdone:
            qdone.add(i)
            jobs.append(("q", i))

    need_q(units[0][1])
    jobs += [("v", 0, nb // 2), ("v", nb // 2, nb // 2)]
    for t in range(n + look + slag):
        if t + qlead < n:
            need_q(units[t + qlead][1])
        if t < n:
            need_q(units[t][1])
            jobs.append(("p1",) + units[t])
        if 0 <= t - look < n:
            jobs.append(("p2",) + units[t - look])
        if t >= look + slag:
            jobs.append(("st",) + units[t - look - slag])
    return jobs


def _kernel(x_hbm, ckv_hbm, wq_hbm, wuk_hbm, wuv_hbm, wo_hbm, wr_hbm, wg_hbm,
            wu_hbm, wd_hbm, c_hbm, wmod_hbm, out_hbm,
            x_v, ckv_v, wq_v, wuk_v, wuv_v, wo_v, wr_v, wg_v, wu_v, wd_v,
            c_v, wmod_v, k_s, v_s, hc_s, x1_s, h2_s, out_s, mod_s,
            sems, wsems, osems):
    S, M = x_v.shape
    NP, _, D = wq_v.shape
    nb = S // T
    qscale = D ** -0.5 * LOG2E
    r0 = S // 4

    plain = {
        "ckv0": (ckv_hbm.at[pl.ds(0, r0)], ckv_v.at[pl.ds(0, r0)]),
        "ckv1": (ckv_hbm.at[pl.ds(r0, S - r0)], ckv_v.at[pl.ds(r0, S - r0)]),
        "x": (x_hbm, x_v), "wo": (wo_hbm, wo_v), "wr": (wr_hbm, wr_v),
        "wg": (wg_hbm, wg_v), "wu": (wu_hbm, wu_v), "wd": (wd_hbm, wd_v),
        "c": (c_hbm, c_v), "wmod": (wmod_hbm, wmod_v),
    }
    cp = {n: pltpu.make_async_copy(s, d, sems.at[i])
          for i, (n, (s, d)) in enumerate(plain.items())}
    for a, (n, s, d) in enumerate((("wuk", wuk_hbm, wuk_v), ("wq", wq_hbm, wq_v),
                                   ("wuv", wuv_hbm, wuv_v))):
        for j in range(NP):
            cp[n, j] = pltpu.make_async_copy(
                s.bitcast(U32).at[:, j, 0], d.at[j], wsems.at[a * NP + j])

    def start(*ns):
        for n in ns:
            cp[n].start()

    def wait(*ns):
        for n in ns:
            cp[n].wait()

    def rng(n, lo, hi):
        return [(n, j) for j in range(lo, hi)]

    def kproj(pairs, lo, n, side=()):
        for a, j in enumerate(pairs):
            w = _unzip(wuk_v[j])
            for e in (0, 1):
                _st(k_s, (2 * j + e,), lo, jnp.dot(
                    ckv_v[lo:lo + n, :], w[:, e * D:(e + 1) * D],
                    preferred_element_type=F32))
                b, nd = 2 * a + e, 2 * len(pairs)
                for job in side[len(side) * b // nd:len(side) * (b + 1) // nd]:
                    job()

    col = {}

    def silu_col():
        c = c_v[...].astype(F32)
        col["c"] = jnp.broadcast_to(_rb(c * _sigmoid(c)), (T, M)).T

    def mod_tile(j):
        p, o = divmod(j * T, M)
        w = wmod_v[:, j * T:(j + 1) * T].astype(F32)
        m = _rb(jnp.sum(w * col["c"], axis=0, keepdims=True))
        if p in (1, 4):
            m = _rb(1.0 + m)
        mod_s[p:p + 1, o:o + T] = m

    def ln1(i):
        _, cen, var = _moments(x_v[i * T:(i + 1) * T, :].astype(F32))
        h = cen * lax.rsqrt(var + EPS) * mod_s[1:2, :] + mod_s[0:1, :]
        for a in range(M // D):
            _st(hc_s, (2 * NP + a,), i * T, h[:, a * D:(a + 1) * D])

    def ld_wide(lo, hi, i, n=1):
        return pltpu.bitcast(jnp.concatenate(
            [hc_s[a, i * T // 2:(i + n) * T // 2, :] for a in range(lo, hi)], axis=1), BF16)

    start(*rng("wuk", 0, 2), "ckv0")
    start(*rng("wuk", 2, 4), "ckv1")
    wait(*rng("wuk", 0, 2), "ckv0")
    kproj(range(0, 2), 0, r0)
    wait(*rng("wuk", 2, 4))
    start(*rng("wuk", 4, NP), "c", "wmod")
    kproj(range(2, 4), 0, r0)
    wait("ckv1")
    start("x")
    kproj(range(0, 4), r0, S - r0)
    wait(*rng("wuk", 4, NP), "c", "wmod")
    start(*rng("wq", 0, NP), *rng("wuv", 0, NP), "wo")
    kproj(range(4, 9), 0, S,
          [silu_col] + [lambda j=j: mod_tile(j) for j in range(6 * M // T)])
    wait("x")
    start("wr", "wg", "wu", "wd")
    kproj(range(9, NP), 0, S, [lambda i=i: ln1(i) for i in range(nb)])
    wait(*rng("wq", 0, NP), *rng("wuv", 0, NP))

    def pair(j, carry):
        tri = (lax.broadcasted_iota(jnp.int32, (T, T), 1)
               <= lax.broadcasted_iota(jnp.int32, (T, T), 0))
        wq, wuv = _unzip(wq_v[j]), _unzip(wuv_v[j])
        q, st = {}, {}
        for job in _pair_jobs(nb, 1, 1, 2):
            if job[0] == "q":
                i = job[1]
                r = jnp.dot(ld_wide(2 * NP, 2 * NP + M // D, i), wq,
                            preferred_element_type=F32)
                for e in (0, 1):
                    q[e, i] = (r[:, e * D:(e + 1) * D] * qscale).astype(BF16)
            elif job[0] == "v":
                _, i, n = job
                r = jnp.dot(ckv_v[i * T:(i + n) * T, :], wuv, preferred_element_type=F32)
                for e in (0, 1):
                    _st(v_s, (e,), i * T, r[:, e * D:(e + 1) * D])
            elif job[0] == "p1":
                _, e, i = job
                s = lax.dot_general(q.pop((e, i)), _ld(k_s, (2 * j + e,), 0, (i + 1) * T),
                                    NT, preferred_element_type=F32)
                tiles = [s[:, a * T:(a + 1) * T] for a in range(i + 1)]
                tiles[-1] = jnp.where(tri, tiles[-1], MASK)
                m = tiles[0]
                for t in tiles[1:]:
                    m = jnp.maximum(m, t)
                st[e, i] = (jnp.max(m, axis=1, keepdims=True), tiles)
            elif job[0] == "p2":
                _, e, i = job
                m, tiles = st.pop((e, i))
                ps = [jnp.exp2(t - m) for t in tiles]
                l = ps[0]
                for p in ps[1:]:
                    l = l + p
                o = jnp.dot(jnp.concatenate(ps, axis=1).astype(BF16),
                            _ld(v_s, (e,), 0, (i + 1) * T), preferred_element_type=F32)
                st[e, i] = o * _recip(jnp.sum(l, axis=1, keepdims=True))
            else:
                _, e, i = job
                _st(hc_s, (2 * j + e,), i * T, st.pop((e, i)))
        return carry

    lax.fori_loop(0, NP, pair, 0)

    lane = lax.broadcasted_iota(jnp.int32, (8, T), 1)
    per = T // 8
    nkey = S // (8 * T)
    scores = [jnp.zeros((8, T), F32) for _ in range(nkey)]
    ot = nb // NOUT
    out_cp = [pltpu.make_async_copy(out_s.at[pl.ds(j * ot * T, ot * T)],
                                    out_hbm.at[pl.ds(j * ot * T, ot * T)], osems.at[j])
              for j in range(NOUT)]
    todo = [ot] * NOUT

    def finalize(i, w_r):
        rows = slice(i * T, (i + 1) * T)
        attn = x1_s[rows, :]
        x1 = _rb(x_v[rows, :].astype(F32) + mod_s[2:3, :] * attn)
        mean, _, var = _moments(x1)
        rstd = _recip(_rb(jnp.sqrt(_rb(_rb(var) + EPS))))
        h2 = _rb(_rb(x1 - _rb(mean)) * rstd)
        h2 = _rb(_rb(h2 * mod_s[4:5, :]) + mod_s[3:4, :])
        out_s[rows, :] = (x1 + mod_s[5:6, :] * h2).astype(BF16)
        x1_s[rows, :] = x1
        h2_s[rows, :] = h2
        r = jnp.sum(h2 * w_r, axis=1, keepdims=True)
        b, o = divmod(i * per, T)
        for a in range(per):
            scores[b] = jnp.where(lane == o + a, r[8 * a:8 * a + 8], scores[b])
        todo[i // ot] -= 1
        if todo[i // ot] == 0:
            out_cp[i // ot].start()

    def oproj(lo, hi):
        for i in range(lo, hi):
            x1_s[i * T:(i + 1) * T, :] = jnp.dot(
                ld_wide(0, 2 * NP, i), wo_v[...], preferred_element_type=F32)

    wait("wo")
    oproj(0, 11)
    wait("wr")
    w_r = wr_v[...].astype(F32).reshape(1, M)
    oproj(11, 15)
    for i in range(0, 11):
        finalize(i, w_r)
    wait("wg", "wu", "wd")
    oproj(15, 16)
    for i in range(11, 16):
        finalize(i, w_r)

    sub = lax.broadcasted_iota(jnp.int32, (8, T), 0)
    ibits = (S - 1).bit_length()
    keys = []
    for b in range(nkey):
        r = _rb(scores[b])
        u = lax.shift_right_logical(lax.bitcast_convert_type(r, jnp.int32), 16)
        u = jnp.where(u >= 0x8000, 0xFFFF - u, u + 0x8000)
        u = jnp.where(r == 0.0, 0x8000, u)
        u = jnp.where(r != r, 0, u)
        tok = b * 8 * T + 8 * lane + sub
        keys.append(lax.bitcast_convert_type(
            KEY_BASE + (u << ibits) + ((1 << ibits) - 1 - tok), F32))
    best = jnp.zeros((8, T), F32)
    for k in range(TOPK):
        m = keys[0]
        for kk in keys[1:]:
            m = jnp.maximum(m, kk)
        m = jnp.max(jnp.max(m, axis=1, keepdims=True), axis=0, keepdims=True)
        best = jnp.where(sub == k, m, best)
        keys = [jnp.where(kk == m, 0.0, kk) for kk in keys]
    bi = lax.bitcast_convert_type(best, jnp.int32) - KEY_BASE
    u = bi >> ibits
    u = jnp.where(u >= 0x8000, u - 0x8000, 0xFFFF - u)
    r_sel = lax.bitcast_convert_type(u << 16, F32)[:, 0:1]
    tok = (1 << ibits) - 1 - (bi & ((1 << ibits) - 1))
    idx = [jnp.clip(tok[k, 0], 0, S - 1) for k in range(TOPK)]

    xs = jnp.concatenate([x1_s[pl.ds(i, 1), :] for i in idx], axis=0)
    hs = jnp.concatenate([h2_s[pl.ds(i, 1), :] for i in idx], axis=0)
    hb = hs.astype(BF16)
    g = _rb(lax.dot_general(hb, wg_v[...], NT, preferred_element_type=F32))
    up = _rb(lax.dot_general(hb, wu_v[...], NT, preferred_element_type=F32))
    a = (_rb(g * _sigmoid(g)) * up).astype(BF16)
    y = _rb(jnp.dot(a, wd_v[...], preferred_element_type=F32))
    y = _rb(y * _sigmoid(r_sel))
    new = _rb(xs + mod_s[5:6, :] * _rb(hs + y))

    for c_ in out_cp:
        c_.wait()
    row16 = lax.broadcasted_iota(jnp.int32, (16, M), 0)
    base = [pl.multiple_of((i // 16) * 16, 16) for i in idx]
    for k in range(TOPK):
        old = out_s[pl.ds(base[k], 16), :].astype(F32)
        out_s[pl.ds(base[k], 16), :] = jnp.where(
            row16 == idx[k] - base[k], new[k:k + 1, :], old).astype(BF16)
    first = []
    for k in range(TOPK):
        f = True
        for j in range(k):
            f = jnp.logical_and(f, base[j] != base[k])
        first.append(f)
    patch = [pltpu.make_async_copy(out_s.at[pl.ds(base[k], 16)],
                                   out_hbm.at[pl.ds(base[k], 16)], osems.at[NOUT + k])
             for k in range(TOPK)]
    for k in range(TOPK):
        pl.when(first[k])(patch[k].start)
    for k in range(TOPK):
        pl.when(first[k])(patch[k].wait)


@jax.jit
def pallas_adaLN_cond__compressed_kv_cla__moe_arch_mod__prompt_kernel(
    A_x: jax.Array,
    A_c_kv: jax.Array,
    A_w_q: jax.Array,
    A_w_uk: jax.Array,
    A_w_uv: jax.Array,
    A_w_o: jax.Array,
    B_x: jax.Array,
    B_w_r: jax.Array,
    B_w_gate: jax.Array,
    B_w_up: jax.Array,
    B_w_down: jax.Array,
    c: jax.Array,
    w_mod: jax.Array,
):
    del B_x
    B, S, M = A_x.shape
    C = A_c_kv.shape[2]
    _, H, D = A_w_q.shape
    F = B_w_gate.shape[1]
    NP = H // 2
    assert B == 1 and A_c_kv.shape[1] == S and D == T and NP == 16
    vm = pltpu.VMEM
    out = pl.pallas_call(
        _kernel,
        out_shape=jax.ShapeDtypeStruct((S, M), A_x.dtype),
        in_specs=[pl.BlockSpec(memory_space=pltpu.HBM)] * 12,
        out_specs=pl.BlockSpec(memory_space=pltpu.HBM),
        scratch_shapes=[
            vm((S, M), BF16), vm((S, C), BF16), vm((NP, M, D), U32),
            vm((NP, C, D), U32), vm((NP, C, D), U32), vm((H * D, M), BF16),
            vm((M,), BF16), vm((F, M), BF16), vm((F, M), BF16), vm((F, M), BF16),
            vm((1, M), BF16), vm((M, 6 * M), BF16),
            vm((H, S // 2, D), U32), vm((2, S // 2, D), U32),
            vm((H + M // D, S // 2, D), U32), vm((S, M), F32), vm((S, M), F32), vm((S, M), BF16), vm((8, M), F32),
            pltpu.SemaphoreType.DMA((10,)),
            pltpu.SemaphoreType.DMA((3 * NP,)),
            pltpu.SemaphoreType.DMA((NOUT + TOPK,)),
        ],
        compiler_params=pltpu.CompilerParams(
            vmem_limit_bytes=110 * 2 ** 20,
            flags={"XLA_TPU_EVENLY_DISTRIBUTE_CRITICAL_NODES": True}),
        name="adaln_cla_moe",
    )(A_x.reshape(S, M), A_c_kv.reshape(S, C), A_w_q.reshape(M, NP, 2, D),
      A_w_uk.reshape(C, NP, 2, D), A_w_uv.reshape(C, NP, 2, D),
      A_w_o.reshape(H * D, M), B_w_r, B_w_gate.T, B_w_up.T, B_w_down, c, w_mod)
    return out.reshape(B, S, M)
```

```python
import math

import jax
import jax.numpy as jnp
import ml_dtypes
import numpy as np
from jax import lax
import jax.experimental.pallas as pl
import jax.experimental.pallas.tpu as pltpu

F32 = jnp.float32
BF16 = jnp.bfloat16
U32 = jnp.uint32
T = 128
TOPK = 8
NOUT = 4
NT = (((1,), (1,)), ((), ()))
LOG2E = math.log2(math.e)
EPS = float(np.float32(ml_dtypes.bfloat16(1e-05)))
MASK = float(np.float32(ml_dtypes.bfloat16(-1000000000.0))) * LOG2E
KEY_BASE = 0x20000000


def _rb(v):
    return v.astype(BF16).astype(F32)


def _sigmoid(z):
    return _rb(1.0 / _rb(1.0 + _rb(jnp.exp(-z))))


def _recip(v):
    r = pltpu.reciprocal(v, approx=True)
    return r * (2.0 - v * r)


def _moments(x):
    inv_n = 1.0 / x.shape[-1]
    mean = jnp.sum(x, axis=-1, keepdims=True) * inv_n
    cen = x - mean
    return mean, cen, jnp.sum(cen * cen, axis=-1, keepdims=True) * inv_n


def _unzip(u):
    lo = lax.bitcast_convert_type(u << 16, F32)
    hi = lax.bitcast_convert_type(u & np.uint32(0xFFFF0000), F32)
    return jnp.concatenate([lo, hi], axis=1).astype(BF16)


def _ld(ref, lead, lo, n):
    return pltpu.bitcast(ref[lead + (pl.ds(lo // 2, n // 2),)], BF16)


def _st(ref, lead, lo, val):
    ref[lead + (pl.ds(lo // 2, val.shape[0] // 2),)] = pltpu.bitcast(val.astype(BF16), U32)


def _pair_jobs(nb, look, qlead, slag):
    tiles = []
    for a in range(nb // 2):
        tiles += [nb - 1 - a, a]
    tiles = [15, 0, 14, 1, 13, 2, 12, 4, 11, 5, 10, 6, 9, 8, 7, 3]
    units = [(e, i) for i in tiles for e in (0, 1)]
    n = len(units)
    jobs, qdone = [], set()

    def need_q(i):
        if i not in qdone:
            qdone.add(i)
            jobs.append(("q", i))

    need_q(units[0][1])
    jobs += [("v", 0, nb // 2), ("v", nb // 2, nb // 2)]
    for t in range(n + look + slag):
        if t + qlead < n:
            need_q(units[t + qlead][1])
        if t < n:
            need_q(units[t][1])
            jobs.append(("p1",) + units[t])
        if 0 <= t - look < n:
            jobs.append(("p2",) + units[t - look])
        if t >= look + slag:
            jobs.append(("st",) + units[t - look - slag])
    return jobs


def _kernel(x_hbm, ckv_hbm, wq_hbm, wuk_hbm, wuv_hbm, wo_hbm, wr_hbm, wg_hbm,
            wu_hbm, wd_hbm, c_hbm, wmod_hbm, out_hbm,
            x_v, ckv_v, wq_v, wuk_v, wuv_v, wo_v, wmod_v, k_s, v_s, hc_s, x1_s, h2_s, out_s,
            wg_v, wu_v, wd_v, mod_s, wr_v, c_v,
            sems, wsems, osems):
    S, M = x_v.shape
    NP, _, D = wq_v.shape
    nb = S // T
    qscale = D ** -0.5 * LOG2E
    r0 = S // 4

    plain = {
        "ckv0": (ckv_hbm.at[pl.ds(0, r0)], ckv_v.at[pl.ds(0, r0)]),
        "ckv1": (ckv_hbm.at[pl.ds(r0, r0)], ckv_v.at[pl.ds(r0, r0)]),
        "ckv2": (ckv_hbm.at[pl.ds(2 * r0, 2 * r0)], ckv_v.at[pl.ds(2 * r0, 2 * r0)]),
        "x": (x_hbm, x_v), "wo": (wo_hbm, wo_v), "wr": (wr_hbm, wr_v),
        "wg": (wg_hbm, wg_v), "wu": (wu_hbm, wu_v), "wd": (wd_hbm, wd_v),
        "c": (c_hbm, c_v), "wmod": (wmod_hbm, wmod_v),
    }
    cp = {n: pltpu.make_async_copy(s, d, sems.at[i])
          for i, (n, (s, d)) in enumerate(plain.items())}
    paired = {"wuk": (0, wuk_hbm, wuk_v), "wq": (1, wq_hbm, wq_v), "wuv": (2, wuv_hbm, wuv_v)}

    def copy(n):
        if isinstance(n, str):
            return cp[n]
        a, s, d = paired[n[0]]
        return pltpu.make_async_copy(
            s.bitcast(U32).at[:, n[1], 0], d.at[n[1]], wsems.at[a * NP + n[1]])

    def start(*ns):
        for n in ns:
            copy(n).start()

    def wait(*ns):
        for n in ns:
            copy(n).wait()

    def rng(n, lo, hi):
        return [(n, j) for j in range(lo, hi)]

    def kproj(pairs, lo, n, side=()):
        for a, j in enumerate(pairs):
            w = _unzip(wuk_v[j])
            for e in (0, 1):
                _st(k_s, (2 * j + e,), lo, jnp.dot(
                    ckv_v[lo:lo + n, :], w[:, e * D:(e + 1) * D],
                    preferred_element_type=F32))
                b, nd = 2 * a + e, 2 * len(pairs)
                for job in side[len(side) * b // nd:len(side) * (b + 1) // nd]:
                    job()

    col = {}

    def silu_col():
        c = c_v[...].astype(F32)
        col["c"] = jnp.broadcast_to(_rb(c * _sigmoid(c)), (T, M)).T

    def mod_tile(j):
        p, o = divmod(j * T, M)
        w = wmod_v[:, j * T:(j + 1) * T].astype(F32)
        m = _rb(jnp.sum(w * col["c"], axis=0, keepdims=True))
        if p in (1, 4):
            m = _rb(1.0 + m)
        mod_s[p:p + 1, o:o + T] = m

    def ln1(i):
        _, cen, var = _moments(x_v[i * T:(i + 1) * T, :].astype(F32))
        h = cen * lax.rsqrt(var + EPS) * mod_s[1:2, :] + mod_s[0:1, :]
        for a in range(M // D):
            _st(hc_s, (2 * NP + a,), i * T, h[:, a * D:(a + 1) * D])

    def ld_wide(lo, hi, i, n=1):
        return pltpu.bitcast(jnp.concatenate(
            [hc_s[a, i * T // 2:(i + n) * T // 2, :] for a in range(lo, hi)], axis=1), BF16)

    start(*rng("wuk", 0, 2), "ckv0", *rng("wuk", 2, 4), "ckv1")
    wait(*rng("wuk", 0, 2), "ckv0")
    kproj(range(0, 2), 0, r0)
    wait(*rng("wuk", 2, 4), "ckv1")
    start("ckv2", *rng("wuk", 4, 6))
    kproj(range(0, 2), r0, r0)
    kproj(range(2, 4), 0, 2 * r0)
    wait("ckv2", *rng("wuk", 4, 6))
    start("c", "wmod", *rng("wuk", 6, 10))
    kproj(range(0, 4), 2 * r0, 2 * r0)
    kproj(range(4, 6), 0, S)
    wait(*rng("wuk", 6, 10), "c", "wmod")
    start(*rng("wuk", 10, NP), "x")
    kproj(range(6, 10), 0, S,
          [silu_col] + [lambda j=j: mod_tile(j) for j in range(6 * M // T)])
    wait(*rng("wuk", 10, NP), "x")
    start(("wq", 0), ("wuv", 0), "wo", "wr", "wg", "wu", "wd")
    kproj(range(10, NP), 0, S, [lambda i=i: ln1(i) for i in range(nb)])

    def pair(j, carry):
        wait(("wq", j), ("wuv", j))

        @pl.when(j + 1 < NP)
        def _():
            start(("wq", j + 1), ("wuv", j + 1))

        tri = (lax.broadcasted_iota(jnp.int32, (T, T), 1)
               <= lax.broadcasted_iota(jnp.int32, (T, T), 0))
        wq, wuv = _unzip(wq_v[j]), _unzip(wuv_v[j])
        q, st = {}, {}
        for job in _pair_jobs(nb, 1, 1, 2):
            if job[0] == "q":
                i = job[1]
                r = jnp.dot(ld_wide(2 * NP, 2 * NP + M // D, i), wq,
                            preferred_element_type=F32)
                for e in (0, 1):
                    q[e, i] = (r[:, e * D:(e + 1) * D] * qscale).astype(BF16)
            elif job[0] == "v":
                _, i, n = job
                r = jnp.dot(ckv_v[i * T:(i + n) * T, :], wuv, preferred_element_type=F32)
                for e in (0, 1):
                    _st(v_s, (e,), i * T, r[:, e * D:(e + 1) * D])
            elif job[0] == "p1":
                _, e, i = job
                s = lax.dot_general(q.pop((e, i)), _ld(k_s, (2 * j + e,), 0, (i + 1) * T),
                                    NT, preferred_element_type=F32)
                tiles = [s[:, a * T:(a + 1) * T] for a in range(i + 1)]
                tiles[-1] = jnp.where(tri, tiles[-1], MASK)
                m = tiles[0]
                for t in tiles[1:]:
                    m = jnp.maximum(m, t)
                st[e, i] = (jnp.max(m, axis=1, keepdims=True), tiles)
            elif job[0] == "p2":
                _, e, i = job
                m, tiles = st.pop((e, i))
                ps = [jnp.exp2(t - m) for t in tiles]
                l = ps[0]
                for p in ps[1:]:
                    l = l + p
                o = jnp.dot(jnp.concatenate(ps, axis=1).astype(BF16),
                            _ld(v_s, (e,), 0, (i + 1) * T), preferred_element_type=F32)
                st[e, i] = o * _recip(jnp.sum(l, axis=1, keepdims=True))
            else:
                _, e, i = job
                _st(hc_s, (2 * j + e,), i * T, st.pop((e, i)))
        return carry

    lax.fori_loop(0, NP, pair, 0)

    lane = lax.broadcasted_iota(jnp.int32, (8, T), 1)
    per = T // 8
    nkey = S // (8 * T)
    scores = [jnp.zeros((8, T), F32) for _ in range(nkey)]
    ot = nb // NOUT
    out_cp = [pltpu.make_async_copy(out_s.at[pl.ds(j * ot * T, ot * T)],
                                    out_hbm.at[pl.ds(j * ot * T, ot * T)], osems.at[j])
              for j in range(NOUT)]
    todo = [ot] * NOUT

    def finalize(i, w_r):
        rows = slice(i * T, (i + 1) * T)
        attn = x1_s[rows, :]
        x1 = _rb(x_v[rows, :].astype(F32) + mod_s[2:3, :] * attn)
        mean, _, var = _moments(x1)
        rstd = _recip(_rb(jnp.sqrt(_rb(_rb(var) + EPS))))
        h2 = _rb(_rb(x1 - _rb(mean)) * rstd)
        h2 = _rb(_rb(h2 * mod_s[4:5, :]) + mod_s[3:4, :])
        out_s[rows, :] = (x1 + mod_s[5:6, :] * h2).astype(BF16)
        x1_s[rows, :] = x1
        h2_s[rows, :] = h2
        r = jnp.sum(h2 * w_r, axis=1, keepdims=True)
        b, o = divmod(i * per, T)
        for a in range(per):
            scores[b] = jnp.where(lane == o + a, r[8 * a:8 * a + 8], scores[b])
        todo[i // ot] -= 1
        if todo[i // ot] == 0:
            out_cp[i // ot].start()

    def oproj(lo, hi):
        for i in range(lo, hi):
            x1_s[i * T:(i + 1) * T, :] = jnp.dot(
                ld_wide(0, 2 * NP, i), wo_v[...], preferred_element_type=F32)

    wait("wo")
    oproj(0, 11)
    wait("wr")
    w_r = wr_v[...].astype(F32).reshape(1, M)
    oproj(11, 15)
    for i in range(0, 11):
        finalize(i, w_r)
    wait("wg", "wu", "wd")
    oproj(15, 16)
    for i in range(11, 16):
        finalize(i, w_r)

    sub = lax.broadcasted_iota(jnp.int32, (8, T), 0)
    ibits = (S - 1).bit_length()
    keys = []
    for b in range(nkey):
        r = _rb(scores[b])
        u = lax.shift_right_logical(lax.bitcast_convert_type(r, jnp.int32), 16)
        u = jnp.where(u >= 0x8000, 0xFFFF - u, u + 0x8000)
        u = jnp.where(r == 0.0, 0x8000, u)
        u = jnp.where(r != r, 0, u)
        tok = b * 8 * T + 8 * lane + sub
        keys.append(lax.bitcast_convert_type(
            KEY_BASE + (u << ibits) + ((1 << ibits) - 1 - tok), F32))
    best = jnp.zeros((8, T), F32)
    for k in range(TOPK):
        m = keys[0]
        for kk in keys[1:]:
            m = jnp.maximum(m, kk)
        m = jnp.max(jnp.max(m, axis=1, keepdims=True), axis=0, keepdims=True)
        best = jnp.where(sub == k, m, best)
        keys = [jnp.where(kk == m, 0.0, kk) for kk in keys]
    bi = lax.bitcast_convert_type(best, jnp.int32) - KEY_BASE
    u = bi >> ibits
    u = jnp.where(u >= 0x8000, u - 0x8000, 0xFFFF - u)
    r_sel = lax.bitcast_convert_type(u << 16, F32)[:, 0:1]
    tok = (1 << ibits) - 1 - (bi & ((1 << ibits) - 1))
    idx = [jnp.clip(tok[k, 0], 0, S - 1) for k in range(TOPK)]

    xs = jnp.concatenate([x1_s[pl.ds(i, 1), :] for i in idx], axis=0)
    hs = jnp.concatenate([h2_s[pl.ds(i, 1), :] for i in idx], axis=0)
    hb = hs.astype(BF16)
    g = _rb(lax.dot_general(hb, wg_v[...], NT, preferred_element_type=F32))
    up = _rb(lax.dot_general(hb, wu_v[...], NT, preferred_element_type=F32))
    a = (_rb(g * _sigmoid(g)) * up).astype(BF16)
    y = _rb(jnp.dot(a, wd_v[...], preferred_element_type=F32))
    y = _rb(y * _sigmoid(r_sel))
    new = _rb(xs + mod_s[5:6, :] * _rb(hs + y))

    for c_ in out_cp:
        c_.wait()
    row16 = lax.broadcasted_iota(jnp.int32, (16, M), 0)
    base = [pl.multiple_of((i // 16) * 16, 16) for i in idx]
    for k in range(TOPK):
        old = out_s[pl.ds(base[k], 16), :].astype(F32)
        out_s[pl.ds(base[k], 16), :] = jnp.where(
            row16 == idx[k] - base[k], new[k:k + 1, :], old).astype(BF16)
    first = []
    for k in range(TOPK):
        f = True
        for j in range(k):
            f = jnp.logical_and(f, base[j] != base[k])
        first.append(f)
    patch = [pltpu.make_async_copy(out_s.at[pl.ds(base[k], 16)],
                                   out_hbm.at[pl.ds(base[k], 16)], osems.at[NOUT + k])
             for k in range(TOPK)]
    for k in range(TOPK):
        pl.when(first[k])(patch[k].start)
    for k in range(TOPK):
        pl.when(first[k])(patch[k].wait)


@jax.jit
def pallas_adaLN_cond__compressed_kv_cla__moe_arch_mod__prompt_kernel(
    A_x: jax.Array,
    A_c_kv: jax.Array,
    A_w_q: jax.Array,
    A_w_uk: jax.Array,
    A_w_uv: jax.Array,
    A_w_o: jax.Array,
    B_x: jax.Array,
    B_w_r: jax.Array,
    B_w_gate: jax.Array,
    B_w_up: jax.Array,
    B_w_down: jax.Array,
    c: jax.Array,
    w_mod: jax.Array,
):
    del B_x
    B, S, M = A_x.shape
    C = A_c_kv.shape[2]
    _, H, D = A_w_q.shape
    F = B_w_gate.shape[1]
    NP = H // 2
    assert B == 1 and A_c_kv.shape[1] == S and D == T and NP == 16
    vm = pltpu.VMEM
    out = pl.pallas_call(
        _kernel,
        out_shape=jax.ShapeDtypeStruct((S, M), A_x.dtype),
        in_specs=[pl.BlockSpec(memory_space=pltpu.HBM)] * 12,
        out_specs=pl.BlockSpec(memory_space=pltpu.HBM),
        scratch_shapes=[
            vm((S, M), BF16), vm((S, C), BF16), vm((NP, M, D), U32),
            vm((NP, C, D), U32), vm((NP, C, D), U32), vm((H * D, M), BF16),
            vm((M, 6 * M), BF16),
            vm((H, S // 2, D), U32), vm((2, S // 2, D), U32),
            vm((H + M // D, S // 2, D), U32), vm((S, M), F32), vm((S, M), F32), vm((S, M), BF16),
            vm((F, M), BF16), vm((F, M), BF16), vm((F, M), BF16),
            vm((8, M), F32), vm((M,), BF16), vm((1, M), BF16),
            pltpu.SemaphoreType.DMA((11,)),
            pltpu.SemaphoreType.DMA((3 * NP,)),
            pltpu.SemaphoreType.DMA((NOUT + TOPK,)),
        ],
        compiler_params=pltpu.CompilerParams(
            vmem_limit_bytes=110 * 2 ** 20,
            flags={"XLA_TPU_EVENLY_DISTRIBUTE_CRITICAL_NODES": True}),
        name="adaln_cla_moe",
    )(A_x.reshape(S, M), A_c_kv.reshape(S, C), A_w_q.reshape(M, NP, 2, D),
      A_w_uk.reshape(C, NP, 2, D), A_w_uv.reshape(C, NP, 2, D),
      A_w_o.reshape(H * D, M), B_w_r, B_w_gate.T, B_w_up.T, B_w_down, c, w_mod)
    return out.reshape(B, S, M)
```

```python
import math

import jax
import jax.numpy as jnp
import ml_dtypes
import numpy as np
from jax import lax
import jax.experimental.pallas as pl
import jax.experimental.pallas.tpu as pltpu

F32 = jnp.float32
BF16 = jnp.bfloat16
U32 = jnp.uint32
T = 128
TOPK = 8
NT = (((1,), (1,)), ((), ()))
LOG2E = math.log2(math.e)
EPS = float(np.float32(ml_dtypes.bfloat16(1e-05)))
MASK = float(np.float32(ml_dtypes.bfloat16(-1000000000.0))) * LOG2E
KEY_BASE = 0x20000000


def _rb(v):
    return v.astype(BF16).astype(F32)


def _sigmoid(z):
    return _rb(1.0 / _rb(1.0 + _rb(jnp.exp(-z))))


def _recip(v):
    r = pltpu.reciprocal(v, approx=True)
    return r * (2.0 - v * r)


def _moments(x):
    inv_n = 1.0 / x.shape[-1]
    mean = jnp.sum(x, axis=-1, keepdims=True) * inv_n
    cen = x - mean
    return mean, cen, jnp.sum(cen * cen, axis=-1, keepdims=True) * inv_n


def _unzip(u):
    lo = lax.bitcast_convert_type(u << 16, F32)
    hi = lax.bitcast_convert_type(u & np.uint32(0xFFFF0000), F32)
    return jnp.concatenate([lo, hi], axis=1).astype(BF16)


def _ld(ref, lead, lo, n):
    return pltpu.bitcast(ref[lead + (pl.ds(lo // 2, n // 2),)], BF16)


def _st(ref, lead, lo, val):
    ref[lead + (pl.ds(lo // 2, val.shape[0] // 2),)] = pltpu.bitcast(val.astype(BF16), U32)


def _pair_jobs(nb, look, qlead, slag):
    tiles = []
    for a in range(nb // 2):
        tiles += [nb - 1 - a, a]
    tiles = [15, 0, 14, 1, 13, 2, 12, 4, 11, 5, 10, 6, 9, 8, 7, 3]
    units = [(e, i) for i in tiles for e in (0, 1)]
    n = len(units)
    jobs, qdone = [], set()

    def need_q(i):
        if i not in qdone:
            qdone.add(i)
            jobs.append(("q", i))

    need_q(units[0][1])
    jobs += [("v", 0, nb // 2), ("v", nb // 2, nb // 2)]
    for t in range(n + look + slag):
        if t + qlead < n:
            need_q(units[t + qlead][1])
        if t < n:
            need_q(units[t][1])
            jobs.append(("p1",) + units[t])
        if 0 <= t - look < n:
            jobs.append(("p2",) + units[t - look])
        if t >= look + slag:
            jobs.append(("st",) + units[t - look - slag])
    return jobs


def _kernel(x_hbm, ckv_hbm, wq_hbm, wuk_hbm, wuv_hbm, wo_hbm, wr_hbm, wg_hbm,
            wu_hbm, wd_hbm, c_hbm, wmod_hbm, out_hbm,
            x_v, ckv_v, wq_v, wuk_v, wuv_v, wo_v, wmod_v, k_s, v_s, hc_s, x1_s, h2_s, out_s,
            wg_v, wu_v, wd_v, wgt_s, wut_s, mod_s, wr_v, c_v,
            sems):
    S, M = x_v.shape
    NP, _, D = wq_v.shape
    F = wd_v.shape[0]
    nb = S // T
    qscale = D ** -0.5 * LOG2E
    r0 = S // 4

    def rows(src, dst, lo, n):
        return [(src.at[pl.ds(lo, n)], dst.at[pl.ds(lo, n)])]

    def heads(src, dst, js):
        return [(src.bitcast(U32).at[:, j, 0], dst.at[j]) for j in js]

    groups = [
        heads(wuk_hbm, wuk_v, range(0, 2)) + rows(ckv_hbm, ckv_v, 0, r0),
        heads(wuk_hbm, wuk_v, range(2, 4)) + rows(ckv_hbm, ckv_v, r0, r0),
        rows(ckv_hbm, ckv_v, 2 * r0, 2 * r0) + heads(wuk_hbm, wuk_v, range(4, 6)),
        [(c_hbm, c_v), (wmod_hbm, wmod_v)] + heads(wuk_hbm, wuk_v, range(6, 10)),
        heads(wuk_hbm, wuk_v, range(10, NP)) + [(x_hbm, x_v)],
        [(wo_hbm, wo_v), (wg_hbm, wg_v), (wu_hbm, wu_v)],
        [(wr_hbm, wr_v)],
        rows(wd_hbm, wd_v, 0, F // 2),
        rows(wd_hbm, wd_v, F // 2, F // 2),
    ]

    def copies(g):
        return [pltpu.make_async_copy(s, d, sems.at[g]) for s, d in groups[g]]

    def pair_copies(j):
        return [pltpu.make_async_copy(s, d, sems.at[len(groups)])
                for s, d in heads(wq_hbm, wq_v, [j]) + heads(wuv_hbm, wuv_v, [j])]

    def start(cps):
        for c in cps:
            c.start()

    def wait(cps):
        for c in cps:
            c.wait()

    def kproj(pairs, lo, n, side=()):
        for a, j in enumerate(pairs):
            w = _unzip(wuk_v[j])
            for e in (0, 1):
                _st(k_s, (2 * j + e,), lo, jnp.dot(
                    ckv_v[lo:lo + n, :], w[:, e * D:(e + 1) * D],
                    preferred_element_type=F32))
                b, nd = 2 * a + e, 2 * len(pairs)
                for job in side[len(side) * b // nd:len(side) * (b + 1) // nd]:
                    job()

    col = {}

    def silu_col():
        c = c_v[...].astype(F32)
        col["c"] = jnp.broadcast_to(_rb(c * _sigmoid(c)), (T, M)).T

    def mod_tile(j):
        p, o = divmod(j * T, M)
        w = wmod_v[:, j * T:(j + 1) * T].astype(F32)
        m = _rb(jnp.sum(w * col["c"], axis=0, keepdims=True))
        if p in (1, 4):
            m = _rb(1.0 + m)
        mod_s[p:p + 1, o:o + T] = m

    def ln1(i):
        _, cen, var = _moments(x_v[i * T:(i + 1) * T, :].astype(F32))
        h = cen * lax.rsqrt(var + EPS) * mod_s[1:2, :] + mod_s[0:1, :]
        for a in range(M // D):
            _st(hc_s, (2 * NP + a,), i * T, h[:, a * D:(a + 1) * D])

    def ld_wide(lo, hi, i, n=1):
        return pltpu.bitcast(jnp.concatenate(
            [hc_s[a, i * T // 2:(i + n) * T // 2, :] for a in range(lo, hi)], axis=1), BF16)

    start(copies(0) + copies(1))
    wait(copies(0))
    kproj(range(0, 2), 0, r0)
    wait(copies(1))
    start(copies(2))
    kproj(range(0, 2), r0, r0)
    kproj(range(2, 4), 0, 2 * r0)
    wait(copies(2))
    start(copies(3))
    kproj(range(0, 4), 2 * r0, 2 * r0)
    kproj(range(4, 6), 0, S)
    wait(copies(3))
    start(copies(4))
    kproj(range(6, 10), 0, S,
          [silu_col] + [lambda j=j: mod_tile(j) for j in range(6 * M // T)])
    wait(copies(4))
    start(pair_copies(0) + copies(5) + copies(6) + copies(7) + copies(8))
    kproj(range(10, NP), 0, S, [lambda i=i: ln1(i) for i in range(nb)])

    def pair(j, carry):
        wait(pair_copies(j))

        @pl.when(j + 1 < NP)
        def _():
            start(pair_copies(j + 1))

        tri = (lax.broadcasted_iota(jnp.int32, (T, T), 1)
               <= lax.broadcasted_iota(jnp.int32, (T, T), 0))
        wq, wuv = _unzip(wq_v[j]), _unzip(wuv_v[j])
        q, st = {}, {}
        for job in _pair_jobs(nb, 1, 1, 2):
            if job[0] == "q":
                i = job[1]
                r = jnp.dot(ld_wide(2 * NP, 2 * NP + M // D, i), wq,
                            preferred_element_type=F32)
                for e in (0, 1):
                    q[e, i] = (r[:, e * D:(e + 1) * D] * qscale).astype(BF16)
            elif job[0] == "v":
                _, i, n = job
                r = jnp.dot(ckv_v[i * T:(i + n) * T, :], wuv, preferred_element_type=F32)
                for e in (0, 1):
                    _st(v_s, (e,), i * T, r[:, e * D:(e + 1) * D])
            elif job[0] == "p1":
                _, e, i = job
                s = lax.dot_general(q.pop((e, i)), _ld(k_s, (2 * j + e,), 0, (i + 1) * T),
                                    NT, preferred_element_type=F32)
                tiles = [s[:, a * T:(a + 1) * T] for a in range(i + 1)]
                tiles[-1] = jnp.where(tri, tiles[-1], MASK)
                m = tiles[0]
                for t in tiles[1:]:
                    m = jnp.maximum(m, t)
                st[e, i] = (jnp.max(m, axis=1, keepdims=True), tiles)
            elif job[0] == "p2":
                _, e, i = job
                m, tiles = st.pop((e, i))
                ps = [jnp.exp2(t - m) for t in tiles]
                l = ps[0]
                for p in ps[1:]:
                    l = l + p
                o = jnp.dot(jnp.concatenate(ps, axis=1).astype(BF16),
                            _ld(v_s, (e,), 0, (i + 1) * T), preferred_element_type=F32)
                st[e, i] = o * _recip(jnp.sum(l, axis=1, keepdims=True))
            else:
                _, e, i = job
                _st(hc_s, (2 * j + e,), i * T, st.pop((e, i)))
        return carry

    lax.fori_loop(0, NP, pair, 0)

    osem = sems.at[len(groups) + 1]
    lane = lax.broadcasted_iota(jnp.int32, (8, T), 1)
    sub = lax.broadcasted_iota(jnp.int32, (8, T), 0)
    ibits = (S - 1).bit_length()
    imask = (1 << ibits) - 1

    def sort_key(r, tok):
        u = lax.shift_right_logical(lax.bitcast_convert_type(r, jnp.int32), 16)
        u = jnp.where(u >= 0x8000, 0xFFFF - u, u + 0x8000)
        u = jnp.where(r == 0.0, 0x8000, u)
        u = jnp.where(r != r, 0, u)
        return lax.bitcast_convert_type(KEY_BASE + imask - tok + (u << ibits), F32)

    def merge_top(best, cols):
        new = jnp.zeros((8, T), F32)
        for a, col_ in enumerate(cols):
            new = jnp.where(lane == 8 * a + sub, col_, new)
        top = jnp.zeros((8, T), F32)
        for row in (new, jnp.where(lane == sub, best, 0.0)):
            row = jnp.max(row, axis=0, keepdims=True)
            above = [jnp.where(col_ > row, 1.0, 0.0) for col_ in cols + [best]]
            while len(above) > 1:
                above = [sum(above[a + 1:a + 2], above[a]) for a in range(0, len(above), 2)]
            rank = jnp.sum(above[0], axis=0, keepdims=True)
            top = jnp.where(rank == sub.astype(F32), row, top)
        return jnp.broadcast_to(jnp.max(top, axis=1, keepdims=True), (8, T))

    def oproj(lo, hi):
        for i in range(lo, hi):
            x1_s[i * T:(i + 1) * T, :] = jnp.dot(
                ld_wide(0, 2 * NP, i), wo_v[...], preferred_element_type=F32)

    def finalize(lo, hi, best):
        w_r = wr_v[...].astype(F32).reshape(1, M)
        for i in range(lo, hi):
            rs = slice(i * T, (i + 1) * T)
            x1 = _rb(x_v[rs, :].astype(F32) + mod_s[2:3, :] * x1_s[rs, :])
            mean, _, var = _moments(x1)
            rstd = _recip(_rb(jnp.sqrt(_rb(_rb(var) + EPS))))
            h2 = _rb(_rb(x1 - _rb(mean)) * rstd)
            h2 = _rb(_rb(h2 * mod_s[4:5, :]) + mod_s[3:4, :])
            out_s[rs, :] = (x1 + mod_s[5:6, :] * h2).astype(BF16)
            x1_s[rs, :] = x1
            h2_s[rs, :] = h2
            r = jnp.broadcast_to(_rb(jnp.sum(h2 * w_r, axis=1, keepdims=True)), (T, T))
            best = merge_top(best, [sort_key(r[a:a + 8], i * T + a + sub)
                                    for a in range(0, T, 8)])
        return best

    cuts = (0, 9, 13, 15, nb)
    out_cp = [pltpu.make_async_copy(out_s.at[pl.ds(lo * T, (hi - lo) * T)],
                                    out_hbm.at[pl.ds(lo * T, (hi - lo) * T)], osem)
              for lo, hi in zip(cuts, cuts[1:])]
    wait(copies(5))
    oproj(cuts[0], cuts[1])
    wgt_s[...] = wg_v[...].T
    wut_s[...] = wu_v[...].T
    best = jnp.zeros((8, T), F32)
    for n in range(1, len(cuts) - 1):
        wait(copies(5 + n))
        if n > 1:
            out_cp[n - 2].start()
        oproj(cuts[n], cuts[n + 1])
        best = finalize(cuts[n - 1], cuts[n], best)
    out_cp[-2].start()
    best = finalize(cuts[-2], cuts[-1], best)
    out_cp[-1].start()

    bi = lax.bitcast_convert_type(best, jnp.int32) - KEY_BASE
    u = bi >> ibits
    u = jnp.where(u >= 0x8000, u - 0x8000, 0xFFFF - u)
    r_sel = lax.bitcast_convert_type(u << 16, F32)[:, 0:1]
    tok = imask - (bi & imask)
    idx = [tok[k, 0] for k in range(TOPK)]

    xs = jnp.concatenate([x1_s[pl.ds(i, 1), :] for i in idx], axis=0)
    hs = jnp.concatenate([h2_s[pl.ds(i, 1), :] for i in idx], axis=0)
    hb = hs.astype(BF16)
    g = _rb(jnp.dot(hb, wgt_s[...], preferred_element_type=F32))
    up = _rb(jnp.dot(hb, wut_s[...], preferred_element_type=F32))
    a = (_rb(g * _sigmoid(g)) * up).astype(BF16)
    y = _rb(jnp.dot(a, wd_v[...], preferred_element_type=F32))
    y = _rb(y * _sigmoid(r_sel))
    new = _rb(xs + mod_s[5:6, :] * _rb(hs + y))

    wait(out_cp)
    row16 = lax.broadcasted_iota(jnp.int32, (16, M), 0)
    base = [pl.multiple_of(i & ~15, 16) for i in idx]
    for k in range(TOPK):
        old = out_s[pl.ds(base[k], 16), :].astype(F32)
        out_s[pl.ds(base[k], 16), :] = jnp.where(
            row16 == idx[k] - base[k], new[k:k + 1, :], old).astype(BF16)
    first = []
    for k in range(TOPK):
        f = True
        for j in range(k):
            f = jnp.logical_and(f, base[j] != base[k])
        first.append(f)
    patch = [pltpu.make_async_copy(out_s.at[pl.ds(base[k], 16)],
                                   out_hbm.at[pl.ds(base[k], 16)], osem)
             for k in range(TOPK)]
    for k in range(TOPK):
        pl.when(first[k])(patch[k].start)
    for k in range(TOPK):
        pl.when(first[k])(patch[k].wait)


@jax.jit
def pallas_adaLN_cond__compressed_kv_cla__moe_arch_mod__prompt_kernel(
    A_x: jax.Array,
    A_c_kv: jax.Array,
    A_w_q: jax.Array,
    A_w_uk: jax.Array,
    A_w_uv: jax.Array,
    A_w_o: jax.Array,
    B_x: jax.Array,
    B_w_r: jax.Array,
    B_w_gate: jax.Array,
    B_w_up: jax.Array,
    B_w_down: jax.Array,
    c: jax.Array,
    w_mod: jax.Array,
):
    del B_x
    B, S, M = A_x.shape
    C = A_c_kv.shape[2]
    _, H, D = A_w_q.shape
    F = B_w_gate.shape[1]
    NP = H // 2
    assert B == 1 and A_c_kv.shape[1] == S and (S, D, NP) == (2048, T, 16)
    vm = pltpu.VMEM
    out = pl.pallas_call(
        _kernel,
        out_shape=jax.ShapeDtypeStruct((S, M), A_x.dtype),
        in_specs=[pl.BlockSpec(memory_space=pltpu.HBM)] * 12,
        out_specs=pl.BlockSpec(memory_space=pltpu.HBM),
        scratch_shapes=[
            vm((S, M), BF16), vm((S, C), BF16), vm((NP, M, D), U32),
            vm((NP, C, D), U32), vm((NP, C, D), U32), vm((H * D, M), BF16),
            vm((M, 6 * M), BF16),
            vm((H, S // 2, D), U32), vm((2, S // 2, D), U32),
            vm((H + M // D, S // 2, D), U32), vm((S, M), F32), vm((S, M), F32), vm((S, M), BF16),
            vm((F, M), BF16), vm((F, M), BF16), vm((F, M), BF16),
            vm((M, F), BF16), vm((M, F), BF16),
            vm((8, M), F32), vm((M,), BF16), vm((1, M), BF16),
            pltpu.SemaphoreType.DMA((11,)),
        ],
        compiler_params=pltpu.CompilerParams(
            vmem_limit_bytes=110 * 2 ** 20,
            flags={"XLA_TPU_EVENLY_DISTRIBUTE_CRITICAL_NODES": True}),
        name="adaln_cla_moe",
    )(A_x.reshape(S, M), A_c_kv.reshape(S, C), A_w_q.reshape(M, NP, 2, D),
      A_w_uk.reshape(C, NP, 2, D), A_w_uv.reshape(C, NP, 2, D),
      A_w_o.reshape(H * D, M), B_w_r, B_w_gate.T, B_w_up.T, B_w_down, c, w_mod)
    return out.reshape(B, S, M)
```

```python
import math

import jax
import jax.numpy as jnp
import ml_dtypes
import numpy as np
from jax import lax
import jax.experimental.pallas as pl
import jax.experimental.pallas.tpu as pltpu

F32 = jnp.float32
BF16 = jnp.bfloat16
U32 = jnp.uint32
T = 128
TOPK = 8
NT = (((1,), (1,)), ((), ()))
LOG2E = math.log2(math.e)
EPS = float(np.float32(ml_dtypes.bfloat16(1e-05)))
MASK = float(np.float32(ml_dtypes.bfloat16(-1000000000.0))) * LOG2E
KEY_BASE = 0x20000000


def _rb(v):
    return v.astype(BF16).astype(F32)


def _sigmoid(z):
    return _rb(1.0 / _rb(1.0 + _rb(jnp.exp(-z))))


def _recip(v):
    r = pltpu.reciprocal(v, approx=True)
    return r * (2.0 - v * r)


def _moments(x):
    inv_n = 1.0 / x.shape[-1]
    mean = jnp.sum(x, axis=-1, keepdims=True) * inv_n
    cen = x - mean
    return mean, cen, jnp.sum(cen * cen, axis=-1, keepdims=True) * inv_n


def _unzip(u):
    lo = lax.bitcast_convert_type(u << 16, F32)
    hi = lax.bitcast_convert_type(u & np.uint32(0xFFFF0000), F32)
    return jnp.concatenate([lo, hi], axis=1).astype(BF16)


def _ld(ref, lead, lo, n):
    return pltpu.bitcast(ref[lead + (pl.ds(lo // 2, n // 2),)], BF16)


def _st(ref, lead, lo, val):
    ref[lead + (pl.ds(lo // 2, val.shape[0] // 2),)] = pltpu.bitcast(val.astype(BF16), U32)


def _pair_jobs(nb, look, qlead, slag):
    tiles = []
    for a in range(nb // 2):
        tiles += [nb - 1 - a, a]
    tiles = [15, 0, 14, 1, 13, 2, 12, 4, 11, 5, 10, 6, 9, 8, 7, 3]
    units = [(e, i) for i in tiles for e in (0, 1)]
    n = len(units)
    jobs, qdone = [], set()

    def need_q(i):
        if i not in qdone:
            qdone.add(i)
            jobs.append(("q", i))

    need_q(units[0][1])
    jobs += [("v", 0, nb // 2), ("v", nb // 2, nb // 2)]
    for t in range(n + look + slag):
        if t + qlead < n:
            need_q(units[t + qlead][1])
        if t < n:
            need_q(units[t][1])
            jobs.append(("p1",) + units[t])
        if 0 <= t - look < n:
            jobs.append(("p2",) + units[t - look])
        if t >= look + slag:
            jobs.append(("st",) + units[t - look - slag])
    return jobs


def _kernel(x_hbm, ckv_hbm, wq_hbm, wuk_hbm, wuv_hbm, wo_hbm, wr_hbm, wg_hbm,
            wu_hbm, wd_hbm, c_hbm, wmod_hbm, out_hbm,
            x_v, ckv_v, wq_v, wuk_v, wuv_v, wo_v, wmod_v, k_s, v_s, hc_s, x1_s, h2_s, out_s,
            wg_v, wu_v, wd_v, wgt_s, wut_s, mod_s, wr_v, c_v,
            sems):
    S, M = x_v.shape
    NP, _, D = wq_v.shape
    F = wd_v.shape[0]
    nb = S // T
    qscale = D ** -0.5 * LOG2E
    r0 = S // 4

    def rows(src, dst, lo, n):
        return [(src.at[pl.ds(lo, n)], dst.at[pl.ds(lo, n)])]

    def heads(src, dst, js):
        return [(src.bitcast(U32).at[:, j, 0], dst.at[j]) for j in js]

    groups = [
        heads(wuk_hbm, wuk_v, range(0, 2)) + rows(ckv_hbm, ckv_v, 0, r0),
        heads(wuk_hbm, wuk_v, range(2, 4)) + rows(ckv_hbm, ckv_v, r0, r0),
        rows(ckv_hbm, ckv_v, 2 * r0, 2 * r0) + heads(wuk_hbm, wuk_v, range(4, 6)),
        [(c_hbm, c_v), (wmod_hbm, wmod_v)] + heads(wuk_hbm, wuk_v, range(6, 10)),
        heads(wuk_hbm, wuk_v, range(10, NP)) + [(x_hbm, x_v)],
        [(wo_hbm, wo_v), (wg_hbm, wg_v), (wu_hbm, wu_v)],
        [(wr_hbm, wr_v)],
        rows(wd_hbm, wd_v, 0, F // 2),
        rows(wd_hbm, wd_v, F // 2, F // 2),
    ]

    def copies(g):
        return [pltpu.make_async_copy(s, d, sems.at[g]) for s, d in groups[g]]

    def pair_copies(j):
        return [pltpu.make_async_copy(s, d, sems.at[len(groups)])
                for s, d in heads(wq_hbm, wq_v, [j]) + heads(wuv_hbm, wuv_v, [j])]

    def start(cps):
        for c in cps:
            c.start()

    def wait(cps):
        for c in cps:
            c.wait()

    def kproj(pairs, lo, n, side=()):
        for a, j in enumerate(pairs):
            w = _unzip(wuk_v[j])
            for e in (0, 1):
                _st(k_s, (2 * j + e,), lo, jnp.dot(
                    ckv_v[lo:lo + n, :], w[:, e * D:(e + 1) * D],
                    preferred_element_type=F32))
                b, nd = 2 * a + e, 2 * len(pairs)
                for job in side[len(side) * b // nd:len(side) * (b + 1) // nd]:
                    job()

    col = {}

    def silu_col():
        c = c_v[...].astype(F32)
        col["c"] = jnp.broadcast_to(_rb(c * _sigmoid(c)), (T, M)).T

    def mod_tile(j):
        p, o = divmod(j * T, M)
        w = wmod_v[:, j * T:(j + 1) * T].astype(F32)
        m = _rb(jnp.sum(w * col["c"], axis=0, keepdims=True))
        if p in (1, 4):
            m = _rb(1.0 + m)
        mod_s[p:p + 1, o:o + T] = m

    def ln1(i):
        _, cen, var = _moments(x_v[i * T:(i + 1) * T, :].astype(F32))
        h = cen * lax.rsqrt(var + EPS) * mod_s[1:2, :] + mod_s[0:1, :]
        for a in range(M // D):
            _st(hc_s, (2 * NP + a,), i * T, h[:, a * D:(a + 1) * D])

    def ld_wide(lo, hi, i, n=1):
        return pltpu.bitcast(jnp.concatenate(
            [hc_s[a, i * T // 2:(i + n) * T // 2, :] for a in range(lo, hi)], axis=1), BF16)

    start(copies(0) + copies(1))
    wait(copies(0))
    kproj(range(0, 2), 0, r0)
    wait(copies(1))
    start(copies(2))
    kproj(range(0, 2), r0, r0)
    kproj(range(2, 4), 0, 2 * r0)
    wait(copies(2))
    start(copies(3))
    kproj(range(0, 4), 2 * r0, 2 * r0)
    kproj(range(4, 6), 0, S)
    wait(copies(3))
    start(copies(4))
    kproj(range(6, 10), 0, S,
          [silu_col] + [lambda j=j: mod_tile(j) for j in range(6 * M // T)])
    wait(copies(4))
    start(pair_copies(0) + copies(5) + copies(6) + copies(7) + copies(8))
    kproj(range(10, NP), 0, S, [lambda i=i: ln1(i) for i in range(nb)])

    def pair(j, low):
        wait(pair_copies(j))

        @pl.when(j + 1 < NP)
        def _():
            start(pair_copies(j + 1))

        tri = (lax.broadcasted_iota(jnp.int32, (T, T), 1)
               <= lax.broadcasted_iota(jnp.int32, (T, T), 0))
        wq, wuv = _unzip(wq_v[j]), _unzip(wuv_v[j])
        q, st = {}, {}
        for job in _pair_jobs(nb, 1, 1, 2):
            if job[0] == "q":
                i = job[1]
                r = jnp.dot(ld_wide(2 * NP, 2 * NP + M // D, i), wq,
                            preferred_element_type=F32)
                for e in (0, 1):
                    q[e, i] = (r[:, e * D:(e + 1) * D] * qscale).astype(BF16)
            elif job[0] == "v":
                _, i, n = job
                r = jnp.dot(ckv_v[i * T:(i + n) * T, :], wuv, preferred_element_type=F32)
                for e in (0, 1):
                    _st(v_s, (e,), i * T, r[:, e * D:(e + 1) * D])
            elif job[0] == "p1":
                _, e, i = job
                s = lax.dot_general(q.pop((e, i)), _ld(k_s, (2 * j + e,), 0, (i + 1) * T),
                                    NT, preferred_element_type=F32)
                tiles = [s[:, a * T:(a + 1) * T] for a in range(i + 1)]
                tiles[-1] = jnp.where(tri, tiles[-1], MASK)
                m = tiles[0]
                for t in tiles[1:]:
                    m = jnp.maximum(m, t)
                m = jnp.max(m, axis=1, keepdims=True)
                st[e, i] = (m, tiles)
                for a in range(0, T, 8):
                    low = jnp.minimum(low, m[a:a + 8])
            elif job[0] == "p2":
                _, e, i = job
                m, tiles = st.pop((e, i))
                ps = [jnp.exp2(t - m) for t in tiles]
                l = ps[0]
                for p in ps[1:]:
                    l = l + p
                o = jnp.dot(jnp.concatenate(ps, axis=1).astype(BF16),
                            _ld(v_s, (e,), 0, (i + 1) * T), preferred_element_type=F32)
                st[e, i] = o * _recip(jnp.sum(l, axis=1, keepdims=True))
            else:
                _, e, i = job
                _st(hc_s, (2 * j + e,), i * T, st.pop((e, i)))
        return low

    low = lax.fori_loop(0, NP, pair, jnp.zeros((8, T), F32))

    @pl.when(jnp.logical_not(jnp.min(low) >= 0.5 * MASK))
    def _():
        @pl.loop(0, NP)
        def _(j):
            v = jnp.dot(ckv_v[...], _unzip(wuv_v[j]), preferred_element_type=F32)
            for e in (0, 1):
                _st(v_s, (e,), 0, v[:, e * D:(e + 1) * D])

            @pl.loop(0, nb)
            def _(i):
                rs = pl.ds(pl.multiple_of(i * (T // 2), T // 2), T // 2)
                h = pltpu.bitcast(jnp.concatenate(
                    [hc_s[2 * NP + a, rs, :] for a in range(M // D)], axis=1), BF16)
                q = jnp.dot(h, _unzip(wq_v[j]), preferred_element_type=F32) * qscale
                seen = (lax.broadcasted_iota(jnp.int32, (T, S), 1)
                        <= i * T + lax.broadcasted_iota(jnp.int32, (T, S), 0))
                for e in (0, 1):
                    s = lax.dot_general(
                        q[:, e * D:(e + 1) * D].astype(BF16), _ld(k_s, (2 * j + e,), 0, S),
                        NT, preferred_element_type=F32)
                    s = jnp.where(seen, s, MASK)
                    p = jnp.exp2(s - jnp.max(s, axis=1, keepdims=True))
                    o = jnp.dot(p.astype(BF16), _ld(v_s, (e,), 0, S),
                                preferred_element_type=F32)
                    o = o * _recip(jnp.sum(p, axis=1, keepdims=True))
                    hc_s[2 * j + e, rs, :] = pltpu.bitcast(o.astype(BF16), U32)

    osem = sems.at[len(groups) + 1]
    lane = lax.broadcasted_iota(jnp.int32, (8, T), 1)
    sub = lax.broadcasted_iota(jnp.int32, (8, T), 0)
    ibits = (S - 1).bit_length()
    imask = (1 << ibits) - 1

    def sort_key(r, tok):
        u = lax.shift_right_logical(lax.bitcast_convert_type(r, jnp.int32), 16)
        u = jnp.where(u >= 0x8000, 0xFFFF - u, u + 0x8000)
        u = jnp.where(r == 0.0, 0x8000, u)
        u = jnp.where(r != r, 0, u)
        return lax.bitcast_convert_type(KEY_BASE + imask - tok + (u << ibits), F32)

    def merge_top(best, cols):
        new = jnp.zeros((8, T), F32)
        for a, col_ in enumerate(cols):
            new = jnp.where(lane == 8 * a + sub, col_, new)
        top = jnp.zeros((8, T), F32)
        for row in (new, jnp.where(lane == sub, best, 0.0)):
            row = jnp.max(row, axis=0, keepdims=True)
            above = [jnp.where(col_ > row, 1.0, 0.0) for col_ in cols + [best]]
            while len(above) > 1:
                above = [sum(above[a + 1:a + 2], above[a]) for a in range(0, len(above), 2)]
            rank = jnp.sum(above[0], axis=0, keepdims=True)
            top = jnp.where(rank == sub.astype(F32), row, top)
        return jnp.broadcast_to(jnp.max(top, axis=1, keepdims=True), (8, T))

    def oproj(lo, hi):
        for i in range(lo, hi):
            x1_s[i * T:(i + 1) * T, :] = jnp.dot(
                ld_wide(0, 2 * NP, i), wo_v[...], preferred_element_type=F32)

    def finalize(lo, hi, best):
        w_r = wr_v[...].astype(F32).reshape(1, M)
        for i in range(lo, hi):
            rs = slice(i * T, (i + 1) * T)
            x1 = _rb(x_v[rs, :].astype(F32) + mod_s[2:3, :] * x1_s[rs, :])
            mean, _, var = _moments(x1)
            rstd = _recip(_rb(jnp.sqrt(_rb(_rb(var) + EPS))))
            h2 = _rb(_rb(x1 - _rb(mean)) * rstd)
            h2 = _rb(_rb(h2 * mod_s[4:5, :]) + mod_s[3:4, :])
            out_s[rs, :] = (x1 + mod_s[5:6, :] * h2).astype(BF16)
            x1_s[rs, :] = x1
            h2_s[rs, :] = h2
            r = jnp.broadcast_to(_rb(jnp.sum(h2 * w_r, axis=1, keepdims=True)), (T, T))
            best = merge_top(best, [sort_key(r[a:a + 8], i * T + a + sub)
                                    for a in range(0, T, 8)])
        return best

    cuts = (0, 9, 13, 15, nb)
    out_cp = [pltpu.make_async_copy(out_s.at[pl.ds(lo * T, (hi - lo) * T)],
                                    out_hbm.at[pl.ds(lo * T, (hi - lo) * T)], osem)
              for lo, hi in zip(cuts, cuts[1:])]
    wait(copies(5))
    oproj(cuts[0], cuts[1])
    wgt_s[...] = wg_v[...].T
    wut_s[...] = wu_v[...].T
    best = jnp.zeros((8, T), F32)
    for n in range(1, len(cuts) - 1):
        wait(copies(5 + n))
        if n > 1:
            out_cp[n - 2].start()
        oproj(cuts[n], cuts[n + 1])
        best = finalize(cuts[n - 1], cuts[n], best)
    out_cp[-2].start()
    best = finalize(cuts[-2], cuts[-1], best)
    out_cp[-1].start()

    bi = lax.bitcast_convert_type(best, jnp.int32) - KEY_BASE
    u = bi >> ibits
    u = jnp.where(u >= 0x8000, u - 0x8000, 0xFFFF - u)
    r_sel = lax.bitcast_convert_type(u << 16, F32)[:, 0:1]
    tok = imask - (bi & imask)
    idx = [tok[k, 0] for k in range(TOPK)]

    xs = jnp.concatenate([x1_s[pl.ds(i, 1), :] for i in idx], axis=0)
    hs = jnp.concatenate([h2_s[pl.ds(i, 1), :] for i in idx], axis=0)
    hb = hs.astype(BF16)
    g = _rb(jnp.dot(hb, wgt_s[...], preferred_element_type=F32))
    up = _rb(jnp.dot(hb, wut_s[...], preferred_element_type=F32))
    a = (_rb(g * _sigmoid(g)) * up).astype(BF16)
    y = _rb(jnp.dot(a, wd_v[...], preferred_element_type=F32))
    y = _rb(y * _sigmoid(r_sel))
    new = _rb(xs + mod_s[5:6, :] * _rb(hs + y))

    wait(out_cp)
    row16 = lax.broadcasted_iota(jnp.int32, (16, M), 0)
    base = [pl.multiple_of(i & ~15, 16) for i in idx]
    for k in range(TOPK):
        old = out_s[pl.ds(base[k], 16), :].astype(F32)
        out_s[pl.ds(base[k], 16), :] = jnp.where(
            row16 == idx[k] - base[k], new[k:k + 1, :], old).astype(BF16)
    first = []
    for k in range(TOPK):
        f = True
        for j in range(k):
            f = jnp.logical_and(f, base[j] != base[k])
        first.append(f)
    patch = [pltpu.make_async_copy(out_s.at[pl.ds(base[k], 16)],
                                   out_hbm.at[pl.ds(base[k], 16)], osem)
             for k in range(TOPK)]
    for k in range(TOPK):
        pl.when(first[k])(patch[k].start)
    for k in range(TOPK):
        pl.when(first[k])(patch[k].wait)


@jax.jit
def pallas_adaLN_cond__compressed_kv_cla__moe_arch_mod__prompt_kernel(
    A_x: jax.Array,
    A_c_kv: jax.Array,
    A_w_q: jax.Array,
    A_w_uk: jax.Array,
    A_w_uv: jax.Array,
    A_w_o: jax.Array,
    B_x: jax.Array,
    B_w_r: jax.Array,
    B_w_gate: jax.Array,
    B_w_up: jax.Array,
    B_w_down: jax.Array,
    c: jax.Array,
    w_mod: jax.Array,
):
    del B_x
    B, S, M = A_x.shape
    C = A_c_kv.shape[2]
    _, H, D = A_w_q.shape
    F = B_w_gate.shape[1]
    NP = H // 2
    assert B == 1 and A_c_kv.shape[1] == S and (S, D, NP) == (2048, T, 16)
    vm = pltpu.VMEM
    out = pl.pallas_call(
        _kernel,
        out_shape=jax.ShapeDtypeStruct((S, M), A_x.dtype),
        in_specs=[pl.BlockSpec(memory_space=pltpu.HBM)] * 12,
        out_specs=pl.BlockSpec(memory_space=pltpu.HBM),
        scratch_shapes=[
            vm((S, M), BF16), vm((S, C), BF16), vm((NP, M, D), U32),
            vm((NP, C, D), U32), vm((NP, C, D), U32), vm((H * D, M), BF16),
            vm((M, 6 * M), BF16),
            vm((H, S // 2, D), U32), vm((2, S // 2, D), U32),
            vm((H + M // D, S // 2, D), U32), vm((S, M), F32), vm((S, M), F32), vm((S, M), BF16),
            vm((F, M), BF16), vm((F, M), BF16), vm((F, M), BF16),
            vm((M, F), BF16), vm((M, F), BF16),
            vm((8, M), F32), vm((M,), BF16), vm((1, M), BF16),
            pltpu.SemaphoreType.DMA((11,)),
        ],
        compiler_params=pltpu.CompilerParams(
            vmem_limit_bytes=110 * 2 ** 20,
            flags={"XLA_TPU_EVENLY_DISTRIBUTE_CRITICAL_NODES": True}),
        name="adaln_cla_moe",
    )(A_x.reshape(S, M), A_c_kv.reshape(S, C), A_w_q.reshape(M, NP, 2, D),
      A_w_uk.reshape(C, NP, 2, D), A_w_uv.reshape(C, NP, 2, D),
      A_w_o.reshape(H * D, M), B_w_r, B_w_gate.T, B_w_up.T, B_w_down, c, w_mod)
    return out.reshape(B, S, M)
```

```python
import math

import jax
import jax.numpy as jnp
import ml_dtypes
import numpy as np
from jax import lax
import jax.experimental.pallas as pl
import jax.experimental.pallas.tpu as pltpu

F32 = jnp.float32
BF16 = jnp.bfloat16
U32 = jnp.uint32
T = 128
TOPK = 8
NT = (((1,), (1,)), ((), ()))
LOG2E = math.log2(math.e)
EPS = float(np.float32(ml_dtypes.bfloat16(1e-05)))
MASK = float(np.float32(ml_dtypes.bfloat16(-1000000000.0))) * LOG2E
KEY_BASE = 0x20000000


def _rb(v):
    return v.astype(BF16).astype(F32)


def _sigmoid(z):
    return _rb(1.0 / _rb(1.0 + _rb(jnp.exp(-z))))


def _recip(v):
    r = pltpu.reciprocal(v, approx=True)
    return r * (2.0 - v * r)


def _moments(x):
    inv_n = 1.0 / x.shape[-1]
    mean = jnp.sum(x, axis=-1, keepdims=True) * inv_n
    cen = x - mean
    return mean, cen, jnp.sum(cen * cen, axis=-1, keepdims=True) * inv_n


def _unzip(u):
    lo = lax.bitcast_convert_type(u << 16, F32)
    hi = lax.bitcast_convert_type(u & np.uint32(0xFFFF0000), F32)
    return jnp.concatenate([lo, hi], axis=1).astype(BF16)


def _ld(ref, lead, lo, n):
    return pltpu.bitcast(ref[lead + (pl.ds(lo // 2, n // 2),)], BF16)


def _st(ref, lead, lo, val):
    ref[lead + (pl.ds(lo // 2, val.shape[0] // 2),)] = pltpu.bitcast(val.astype(BF16), U32)


def _pair_jobs():
    tiles = (0, 15, 14, 4, 1, 13, 5, 2, 12, 7, 9, 10, 8, 11, 6, 3)
    units = [(e, i) for i in tiles for e in (0, 1)]
    n = len(units)
    jobs = [("q", tiles[0]), ("v",)]
    for t in range(n + 4):
        if t + 1 < n and units[t + 1][0] == 0:
            jobs.append(("q", units[t + 1][1]))
        for name, lag in (("p1", 0), ("p2", 1), ("st", 4)):
            if 0 <= t - lag < n:
                jobs.append((name,) + units[t - lag])
    return jobs


def _kernel(x_hbm, ckv_hbm, wq_hbm, wuk_hbm, wuv_hbm, wo_hbm, wr_hbm, wg_hbm,
            wu_hbm, wd_hbm, c_hbm, wmod_hbm, out_hbm,
            x_v, ckv_v, wq_v, wuk_v, wuv_v, wo_v, wmod_v, k_s, v_s, hc_s, x1_s, h2_s, out_s,
            wg_v, wu_v, wd_v, wgt_s, wut_s, mod_s, wr_v, c_v,
            sems):
    S, M = x_v.shape
    NP, _, D = wq_v.shape
    F = wd_v.shape[0]
    nb = S // T
    qscale = D ** -0.5 * LOG2E
    r0 = S // 4

    def rows(src, dst, lo, n):
        return [(src.at[pl.ds(lo, n)], dst.at[pl.ds(lo, n)])]

    def heads(src, dst, js):
        return [(src.bitcast(U32).at[:, j, 0], dst.at[j]) for j in js]

    groups = [
        heads(wuk_hbm, wuk_v, range(0, 2)) + rows(ckv_hbm, ckv_v, 0, r0),
        heads(wuk_hbm, wuk_v, range(2, 4)) + rows(ckv_hbm, ckv_v, r0, r0),
        rows(ckv_hbm, ckv_v, 2 * r0, 2 * r0) + heads(wuk_hbm, wuk_v, range(4, 6)),
        [(c_hbm, c_v), (wmod_hbm, wmod_v)] + heads(wuk_hbm, wuk_v, range(6, 10)),
        heads(wuk_hbm, wuk_v, range(10, NP)) + [(x_hbm, x_v)],
        [(wo_hbm, wo_v), (wg_hbm, wg_v), (wu_hbm, wu_v)],
        [(wr_hbm, wr_v)],
        rows(wd_hbm, wd_v, 0, F // 2),
        rows(wd_hbm, wd_v, F // 2, F // 2),
    ]

    def copies(g):
        return [pltpu.make_async_copy(s, d, sems.at[g]) for s, d in groups[g]]

    def pair_copies(j):
        return [pltpu.make_async_copy(s, d, sems.at[len(groups)])
                for s, d in heads(wq_hbm, wq_v, [j]) + heads(wuv_hbm, wuv_v, [j])]

    def start(cps):
        for c in cps:
            c.start()

    def wait(cps):
        for c in cps:
            c.wait()

    def kproj(pairs, lo, n, side=()):
        for a, j in enumerate(pairs):
            w = _unzip(wuk_v[j])
            for e in (0, 1):
                _st(k_s, (2 * j + e,), lo, jnp.dot(
                    ckv_v[lo:lo + n, :], w[:, e * D:(e + 1) * D],
                    preferred_element_type=F32))
                b, nd = 2 * a + e, 2 * len(pairs)
                for job in side[len(side) * b // nd:len(side) * (b + 1) // nd]:
                    job()

    col = {}

    def silu_col():
        c = c_v[...].astype(F32)
        col["c"] = jnp.broadcast_to(_rb(c * _sigmoid(c)), (T, M)).T

    def mod_tile(j):
        p, o = divmod(j * T, M)
        w = wmod_v[:, j * T:(j + 1) * T].astype(F32)
        m = _rb(jnp.sum(w * col["c"], axis=0, keepdims=True))
        if p in (1, 4):
            m = _rb(1.0 + m)
        mod_s[p:p + 1, o:o + T] = m

    def ln1(i):
        _, cen, var = _moments(x_v[i * T:(i + 1) * T, :].astype(F32))
        h = cen * lax.rsqrt(var + EPS) * mod_s[1:2, :] + mod_s[0:1, :]
        for a in range(M // D):
            _st(hc_s, (2 * NP + a,), i * T, h[:, a * D:(a + 1) * D])

    def ld_wide(lo, hi, i, n=1):
        return pltpu.bitcast(jnp.concatenate(
            [hc_s[a, i * T // 2:(i + n) * T // 2, :] for a in range(lo, hi)], axis=1), BF16)

    start(copies(0) + copies(1))
    wait(copies(0))
    kproj(range(0, 2), 0, r0)
    wait(copies(1))
    start(copies(2))
    kproj(range(0, 2), r0, r0)
    kproj(range(2, 4), 0, 2 * r0)
    wait(copies(2))
    start(copies(3))
    kproj(range(0, 4), 2 * r0, 2 * r0)
    kproj(range(4, 6), 0, S)
    wait(copies(3))
    start(copies(4))
    kproj(range(6, 10), 0, S,
          [silu_col] + [lambda j=j: mod_tile(j) for j in range(6 * M // T)])
    wait(copies(4))
    start(pair_copies(0) + copies(5) + copies(6) + copies(7) + copies(8))
    kproj(range(10, NP), 0, S, [lambda i=i: ln1(i) for i in range(nb)])

    def pair(j, low):
        wait(pair_copies(j))

        @pl.when(j + 1 < NP)
        def _():
            start(pair_copies(j + 1))

        tri = (lax.broadcasted_iota(jnp.int32, (T, T), 1)
               <= lax.broadcasted_iota(jnp.int32, (T, T), 0))
        wq, wuv = _unzip(wq_v[j]), _unzip(wuv_v[j])
        q, st = {}, {}
        for job in _pair_jobs():
            if job[0] == "q":
                i = job[1]
                r = jnp.dot(ld_wide(2 * NP, 2 * NP + M // D, i), wq,
                            preferred_element_type=F32)
                for e in (0, 1):
                    q[e, i] = (r[:, e * D:(e + 1) * D] * qscale).astype(BF16)
            elif job[0] == "v":
                r = jnp.dot(ckv_v[...], wuv, preferred_element_type=F32)
                for e in (0, 1):
                    _st(v_s, (e,), 0, r[:, e * D:(e + 1) * D])
            elif job[0] == "p1":
                _, e, i = job
                s = lax.dot_general(q.pop((e, i)), _ld(k_s, (2 * j + e,), 0, (i + 1) * T),
                                    NT, preferred_element_type=F32)
                tiles = [s[:, a * T:(a + 1) * T] for a in range(i + 1)]
                tiles[-1] = jnp.where(tri, tiles[-1], MASK)
                m = tiles[0]
                for t in tiles[1:]:
                    m = jnp.maximum(m, t)
                m = jnp.max(m, axis=1, keepdims=True)
                st[e, i] = (m, tiles)
                for a in range(0, T, 8):
                    low = jnp.minimum(low, m[a:a + 8])
            elif job[0] == "p2":
                _, e, i = job
                m, tiles = st.pop((e, i))
                ps = [jnp.exp2(t - m) for t in tiles]
                l = ps[0]
                for p in ps[1:]:
                    l = l + p
                o = jnp.dot(jnp.concatenate(ps, axis=1).astype(BF16),
                            _ld(v_s, (e,), 0, (i + 1) * T), preferred_element_type=F32)
                st[e, i] = o * _recip(jnp.sum(l, axis=1, keepdims=True))
            else:
                _, e, i = job
                _st(hc_s, (2 * j + e,), i * T, st.pop((e, i)))
        return low

    low = lax.fori_loop(0, NP, pair, jnp.zeros((8, T), F32))

    @pl.when(jnp.logical_not(jnp.min(low) >= 0.5 * MASK))
    def _():
        @pl.loop(0, NP)
        def _(j):
            v = jnp.dot(ckv_v[...], _unzip(wuv_v[j]), preferred_element_type=F32)
            for e in (0, 1):
                _st(v_s, (e,), 0, v[:, e * D:(e + 1) * D])

            @pl.loop(0, nb)
            def _(i):
                rs = pl.ds(pl.multiple_of(i * (T // 2), T // 2), T // 2)
                h = pltpu.bitcast(jnp.concatenate(
                    [hc_s[2 * NP + a, rs, :] for a in range(M // D)], axis=1), BF16)
                q = jnp.dot(h, _unzip(wq_v[j]), preferred_element_type=F32) * qscale
                seen = (lax.broadcasted_iota(jnp.int32, (T, S), 1)
                        <= i * T + lax.broadcasted_iota(jnp.int32, (T, S), 0))
                for e in (0, 1):
                    s = lax.dot_general(
                        q[:, e * D:(e + 1) * D].astype(BF16), _ld(k_s, (2 * j + e,), 0, S),
                        NT, preferred_element_type=F32)
                    s = jnp.where(seen, s, MASK)
                    p = jnp.exp2(s - jnp.max(s, axis=1, keepdims=True))
                    o = jnp.dot(p.astype(BF16), _ld(v_s, (e,), 0, S),
                                preferred_element_type=F32)
                    o = o * _recip(jnp.sum(p, axis=1, keepdims=True))
                    hc_s[2 * j + e, rs, :] = pltpu.bitcast(o.astype(BF16), U32)

    osem = sems.at[len(groups) + 1]
    lane = lax.broadcasted_iota(jnp.int32, (8, T), 1)
    sub = lax.broadcasted_iota(jnp.int32, (8, T), 0)
    ibits = (S - 1).bit_length()
    imask = (1 << ibits) - 1

    def sort_key(r, tok):
        u = lax.shift_right_logical(lax.bitcast_convert_type(r, jnp.int32), 16)
        u = jnp.where(u >= 0x8000, 0xFFFF - u, u + 0x8000)
        u = jnp.where(r == 0.0, 0x8000, u)
        u = jnp.where(r != r, 0, u)
        return lax.bitcast_convert_type(KEY_BASE + imask - tok + (u << ibits), F32)

    def merge_top(best, cols):
        new = jnp.zeros((8, T), F32)
        for a, col_ in enumerate(cols):
            new = jnp.where(lane == 8 * a + sub, col_, new)
        top = jnp.zeros((8, T), F32)
        for row in (new, jnp.where(lane == sub, best, 0.0)):
            row = jnp.max(row, axis=0, keepdims=True)
            above = [jnp.where(col_ > row, 1.0, 0.0) for col_ in cols + [best]]
            while len(above) > 1:
                above = [sum(above[a + 1:a + 2], above[a]) for a in range(0, len(above), 2)]
            rank = jnp.sum(above[0], axis=0, keepdims=True)
            top = jnp.where(rank == sub.astype(F32), row, top)
        return jnp.broadcast_to(jnp.max(top, axis=1, keepdims=True), (8, T))

    def oproj(lo, hi):
        for i in range(lo, hi):
            x1_s[i * T:(i + 1) * T, :] = jnp.dot(
                ld_wide(0, 2 * NP, i), wo_v[...], preferred_element_type=F32)

    def finalize(lo, hi, best):
        w_r = wr_v[...].astype(F32).reshape(1, M)
        for i in range(lo, hi):
            rs = slice(i * T, (i + 1) * T)
            x1 = _rb(x_v[rs, :].astype(F32) + mod_s[2:3, :] * x1_s[rs, :])
            mean, _, var = _moments(x1)
            rstd = _recip(_rb(jnp.sqrt(_rb(_rb(var) + EPS))))
            h2 = _rb(_rb(x1 - _rb(mean)) * rstd)
            h2 = _rb(_rb(h2 * mod_s[4:5, :]) + mod_s[3:4, :])
            out_s[rs, :] = (x1 + mod_s[5:6, :] * h2).astype(BF16)
            x1_s[rs, :] = x1
            h2_s[rs, :] = h2
            r = jnp.broadcast_to(_rb(jnp.sum(h2 * w_r, axis=1, keepdims=True)), (T, T))
            best = merge_top(best, [sort_key(r[a:a + 8], i * T + a + sub)
                                    for a in range(0, T, 8)])
        return best

    cuts = (0, 9, 13, 15, nb)
    out_cp = [pltpu.make_async_copy(out_s.at[pl.ds(lo * T, (hi - lo) * T)],
                                    out_hbm.at[pl.ds(lo * T, (hi - lo) * T)], osem)
              for lo, hi in zip(cuts, cuts[1:])]
    wait(copies(5))
    oproj(cuts[0], cuts[1])
    wgt_s[...] = wg_v[...].T
    wut_s[...] = wu_v[...].T
    best = jnp.zeros((8, T), F32)
    for n in range(1, len(cuts) - 1):
        wait(copies(5 + n))
        if n > 1:
            out_cp[n - 2].start()
        oproj(cuts[n], cuts[n + 1])
        best = finalize(cuts[n - 1], cuts[n], best)
    out_cp[-2].start()
    best = finalize(cuts[-2], cuts[-1], best)
    out_cp[-1].start()

    bi = lax.bitcast_convert_type(best, jnp.int32) - KEY_BASE
    u = bi >> ibits
    u = jnp.where(u >= 0x8000, u - 0x8000, 0xFFFF - u)
    r_sel = lax.bitcast_convert_type(u << 16, F32)[:, 0:1]
    tok = imask - (bi & imask)
    idx = [tok[k, 0] for k in range(TOPK)]

    xs = jnp.concatenate([x1_s[pl.ds(i, 1), :] for i in idx], axis=0)
    hs = jnp.concatenate([h2_s[pl.ds(i, 1), :] for i in idx], axis=0)
    hb = hs.astype(BF16)
    g = _rb(jnp.dot(hb, wgt_s[...], preferred_element_type=F32))
    up = _rb(jnp.dot(hb, wut_s[...], preferred_element_type=F32))
    a = (_rb(g * _sigmoid(g)) * up).astype(BF16)
    y = _rb(jnp.dot(a, wd_v[...], preferred_element_type=F32))
    y = _rb(y * _sigmoid(r_sel))
    new = _rb(xs + mod_s[5:6, :] * _rb(hs + y))

    wait(out_cp)
    row16 = lax.broadcasted_iota(jnp.int32, (16, M), 0)
    base = [pl.multiple_of(i & ~15, 16) for i in idx]
    for k in range(TOPK):
        old = out_s[pl.ds(base[k], 16), :].astype(F32)
        out_s[pl.ds(base[k], 16), :] = jnp.where(
            row16 == idx[k] - base[k], new[k:k + 1, :], old).astype(BF16)
    first = []
    for k in range(TOPK):
        f = True
        for j in range(k):
            f = jnp.logical_and(f, base[j] != base[k])
        first.append(f)
    patch = [pltpu.make_async_copy(out_s.at[pl.ds(base[k], 16)],
                                   out_hbm.at[pl.ds(base[k], 16)], osem)
             for k in range(TOPK)]
    for k in range(TOPK):
        pl.when(first[k])(patch[k].start)
    for k in range(TOPK):
        pl.when(first[k])(patch[k].wait)


@jax.jit
def pallas_adaLN_cond__compressed_kv_cla__moe_arch_mod__prompt_kernel(
    A_x: jax.Array,
    A_c_kv: jax.Array,
    A_w_q: jax.Array,
    A_w_uk: jax.Array,
    A_w_uv: jax.Array,
    A_w_o: jax.Array,
    B_x: jax.Array,
    B_w_r: jax.Array,
    B_w_gate: jax.Array,
    B_w_up: jax.Array,
    B_w_down: jax.Array,
    c: jax.Array,
    w_mod: jax.Array,
):
    del B_x
    B, S, M = A_x.shape
    C = A_c_kv.shape[2]
    _, H, D = A_w_q.shape
    F = B_w_gate.shape[1]
    NP = H // 2
    assert B == 1 and A_c_kv.shape[1] == S and (S, D, NP) == (2048, T, 16)
    vm = pltpu.VMEM
    out = pl.pallas_call(
        _kernel,
        out_shape=jax.ShapeDtypeStruct((S, M), A_x.dtype),
        in_specs=[pl.BlockSpec(memory_space=pltpu.HBM)] * 12,
        out_specs=pl.BlockSpec(memory_space=pltpu.HBM),
        scratch_shapes=[
            vm((S, M), BF16), vm((S, C), BF16), vm((NP, M, D), U32),
            vm((NP, C, D), U32), vm((NP, C, D), U32), vm((H * D, M), BF16),
            vm((M, 6 * M), BF16),
            vm((H, S // 2, D), U32), vm((2, S // 2, D), U32),
            vm((H + M // D, S // 2, D), U32), vm((S, M), F32), vm((S, M), F32), vm((S, M), BF16),
            vm((F, M), BF16), vm((F, M), BF16), vm((F, M), BF16),
            vm((M, F), BF16), vm((M, F), BF16),
            vm((8, M), F32), vm((M,), BF16), vm((1, M), BF16),
            pltpu.SemaphoreType.DMA((11,)),
        ],
        compiler_params=pltpu.CompilerParams(
            vmem_limit_bytes=110 * 2 ** 20, disable_bounds_checks=True,
            flags={"XLA_TPU_EVENLY_DISTRIBUTE_CRITICAL_NODES": True}),
        name="adaln_cla_moe",
    )(A_x.reshape(S, M), A_c_kv.reshape(S, C), A_w_q.reshape(M, NP, 2, D),
      A_w_uk.reshape(C, NP, 2, D), A_w_uv.reshape(C, NP, 2, D),
      A_w_o.reshape(H * D, M), B_w_r, B_w_gate.T, B_w_up.T, B_w_down, c, w_mod)
    return out.reshape(B, S, M)
```

```python
import math

import jax
import jax.numpy as jnp
import numpy as np
from jax import lax
import jax.experimental.pallas as pl
import jax.experimental.pallas.tpu as pltpu

F32 = jnp.float32
BF16 = jnp.bfloat16
U32 = jnp.uint32
T = 128
TOPK = 8
NT = (((1,), (1,)), ((), ()))
LOG2E = math.log2(math.e)
EPS = 1.0013580322265625e-05
MASK = -998244352.0 * LOG2E
KEY_BASE = 0x20000000


def _rb(v):
    return v.astype(BF16).astype(F32)


def _sigmoid(z):
    return _rb(1.0 / _rb(1.0 + _rb(jnp.exp(-z))))


def _recip(v):
    r = pltpu.reciprocal(v, approx=True)
    return r * (2.0 - v * r)


def _moments(x):
    inv_n = 1.0 / x.shape[-1]
    mean = jnp.sum(x, axis=-1, keepdims=True) * inv_n
    cen = x - mean
    return mean, cen, jnp.sum(cen * cen, axis=-1, keepdims=True) * inv_n


def _unzip(u):
    lo = lax.bitcast_convert_type(u << 16, F32)
    hi = lax.bitcast_convert_type(u & np.uint32(0xFFFF0000), F32)
    return jnp.concatenate([lo, hi], axis=1).astype(BF16)


def _ld(ref, lead, lo, n):
    return pltpu.bitcast(ref[lead + (pl.ds(lo // 2, n // 2),)], BF16)


def _st(ref, lead, lo, val):
    ref[lead + (pl.ds(lo // 2, val.shape[0] // 2),)] = pltpu.bitcast(val.astype(BF16), U32)


def _pair_jobs():
    tiles = (0, 15, 14, 4, 1, 13, 5, 2, 12, 7, 9, 10, 8, 11, 6, 3)
    units = [(e, i) for i in tiles for e in (0, 1)]
    n = len(units)
    jobs = [("q", tiles[0]), ("v",)]
    for t in range(n + 4):
        if t + 1 < n and units[t + 1][0] == 0:
            jobs.append(("q", units[t + 1][1]))
        for name, lag in (("p1", 0), ("p2", 1), ("st", 4)):
            if 0 <= t - lag < n:
                jobs.append((name,) + units[t - lag])
    return jobs


def _kernel(x_hbm, ckv_hbm, wq_hbm, wuk_hbm, wuv_hbm, wo_hbm, wr_hbm, wg_hbm,
            wu_hbm, wd_hbm, c_hbm, wmod_hbm, out_hbm,
            x_v, ckv_v, wq_v, wuk_v, wuv_v, wo_v, wmod_v, k_s, v_s, hc_s, x1_s, h2_s, out_s,
            wg_v, wu_v, wd_v, wgt_s, wut_s, mod_s, wr_v, c_v,
            sems):
    S, M = x_v.shape
    NP, _, D = wq_v.shape
    F = wd_v.shape[0]
    nb = S // T
    qscale = D ** -0.5 * LOG2E
    r0 = S // 4

    def rows(src, dst, lo, n):
        return [(src.at[pl.ds(lo, n)], dst.at[pl.ds(lo, n)])]

    def heads(src, dst, js):
        return [(src.bitcast(U32).at[:, j, 0], dst.at[j]) for j in js]

    groups = [
        heads(wuk_hbm, wuk_v, range(0, 2)) + rows(ckv_hbm, ckv_v, 0, r0),
        heads(wuk_hbm, wuk_v, range(2, 4)) + rows(ckv_hbm, ckv_v, r0, r0),
        rows(ckv_hbm, ckv_v, 2 * r0, 2 * r0) + heads(wuk_hbm, wuk_v, range(4, 6)),
        [(c_hbm, c_v), (wmod_hbm, wmod_v)] + heads(wuk_hbm, wuk_v, range(6, 10)),
        heads(wuk_hbm, wuk_v, range(10, NP)) + [(x_hbm, x_v)],
        [(wo_hbm, wo_v), (wg_hbm, wg_v), (wu_hbm, wu_v)],
        [(wr_hbm, wr_v)],
        rows(wd_hbm, wd_v, 0, F // 2),
        rows(wd_hbm, wd_v, F // 2, F // 2),
    ]

    def copies(g):
        return [pltpu.make_async_copy(s, d, sems.at[g]) for s, d in groups[g]]

    def pair_copies(j):
        return [pltpu.make_async_copy(s, d, sems.at[len(groups)])
                for s, d in heads(wq_hbm, wq_v, [j]) + heads(wuv_hbm, wuv_v, [j])]

    def start(cps):
        for c in cps:
            c.start()

    def wait(cps):
        for c in cps:
            c.wait()

    def kproj(pairs, lo, n, side=()):
        for a, j in enumerate(pairs):
            w = _unzip(wuk_v[j])
            for e in (0, 1):
                _st(k_s, (2 * j + e,), lo, jnp.dot(
                    ckv_v[lo:lo + n, :], w[:, e * D:(e + 1) * D],
                    preferred_element_type=F32))
                b, nd = 2 * a + e, 2 * len(pairs)
                for job in side[len(side) * b // nd:len(side) * (b + 1) // nd]:
                    job()

    col = {}

    def silu_col():
        c = c_v[...].astype(F32)
        col["c"] = jnp.broadcast_to(_rb(c * _sigmoid(c)), (T, M)).T

    def mod_tile(j):
        p, o = divmod(j * T, M)
        w = wmod_v[:, j * T:(j + 1) * T].astype(F32)
        m = _rb(jnp.sum(w * col["c"], axis=0, keepdims=True))
        if p in (1, 4):
            m = _rb(1.0 + m)
        mod_s[p:p + 1, o:o + T] = m

    def ln1(i):
        _, cen, var = _moments(x_v[i * T:(i + 1) * T, :].astype(F32))
        h = cen * lax.rsqrt(var + EPS) * mod_s[1:2, :] + mod_s[0:1, :]
        for a in range(M // D):
            _st(hc_s, (2 * NP + a,), i * T, h[:, a * D:(a + 1) * D])

    def ld_wide(lo, hi, i):
        return pltpu.bitcast(jnp.concatenate(
            [hc_s[a, i * T // 2:(i + 1) * T // 2, :] for a in range(lo, hi)], axis=1), BF16)

    start(copies(0) + copies(1))
    wait(copies(0))
    kproj(range(0, 2), 0, r0)
    wait(copies(1))
    start(copies(2))
    kproj(range(0, 2), r0, r0)
    kproj(range(2, 4), 0, 2 * r0)
    wait(copies(2))
    start(copies(3))
    kproj(range(0, 4), 2 * r0, 2 * r0)
    kproj(range(4, 6), 0, S)
    wait(copies(3))
    start(copies(4))
    kproj(range(6, 10), 0, S,
          [silu_col] + [lambda j=j: mod_tile(j) for j in range(6 * M // T)])
    wait(copies(4))
    start(pair_copies(0) + copies(5) + copies(6) + copies(7) + copies(8))
    kproj(range(10, NP), 0, S, [lambda i=i: ln1(i) for i in range(nb)])

    def pair(j, low):
        wait(pair_copies(j))

        @pl.when(j + 1 < NP)
        def _():
            start(pair_copies(j + 1))

        tri = (lax.broadcasted_iota(jnp.int32, (T, T), 1)
               <= lax.broadcasted_iota(jnp.int32, (T, T), 0))
        wq, wuv = _unzip(wq_v[j]), _unzip(wuv_v[j])
        q, st = {}, {}
        for job in _pair_jobs():
            if job[0] == "q":
                i = job[1]
                r = jnp.dot(ld_wide(2 * NP, 2 * NP + M // D, i), wq,
                            preferred_element_type=F32)
                for e in (0, 1):
                    q[e, i] = (r[:, e * D:(e + 1) * D] * qscale).astype(BF16)
            elif job[0] == "v":
                r = jnp.dot(ckv_v[...], wuv, preferred_element_type=F32)
                for e in (0, 1):
                    _st(v_s, (e,), 0, r[:, e * D:(e + 1) * D])
            elif job[0] == "p1":
                _, e, i = job
                s = lax.dot_general(q.pop((e, i)), _ld(k_s, (2 * j + e,), 0, (i + 1) * T),
                                    NT, preferred_element_type=F32)
                tiles = [s[:, a * T:(a + 1) * T] for a in range(i + 1)]
                tiles[-1] = jnp.where(tri, tiles[-1], MASK)
                m = tiles[0]
                for t in tiles[1:]:
                    m = jnp.maximum(m, t)
                m = jnp.max(m, axis=1, keepdims=True)
                st[e, i] = (m, tiles)
                for a in range(0, T, 8):
                    low = jnp.minimum(low, m[a:a + 8])
            elif job[0] == "p2":
                _, e, i = job
                m, tiles = st.pop((e, i))
                ps = [jnp.exp2(t - m) for t in tiles]
                l = ps[0]
                for p in ps[1:]:
                    l = l + p
                o = jnp.dot(jnp.concatenate(ps, axis=1).astype(BF16),
                            _ld(v_s, (e,), 0, (i + 1) * T), preferred_element_type=F32)
                st[e, i] = o * _recip(jnp.sum(l, axis=1, keepdims=True))
            else:
                _, e, i = job
                _st(hc_s, (2 * j + e,), i * T, st.pop((e, i)))
        return low

    low = lax.fori_loop(0, NP, pair, jnp.zeros((8, T), F32))

    @pl.when(jnp.logical_not(jnp.min(low) >= 0.5 * MASK))
    def _():
        @pl.loop(0, 2 * NP)
        def _(hd):
            def weight(ref):
                w = _unzip(ref[hd // 2]).astype(F32)
                return jnp.where(hd % 2 == 0, w[:, :D], w[:, D:]).astype(BF16)

            def words(i):
                return pl.ds(pl.multiple_of(i * (T // 2), T // 2), T // 2)

            @pl.loop(0, nb)
            def _(i):
                v = jnp.dot(ckv_v[pl.ds(pl.multiple_of(i * T, T), T), :], weight(wuv_v),
                            preferred_element_type=F32)
                v_s[0, words(i), :] = pltpu.bitcast(v.astype(BF16), U32)

            @pl.loop(0, nb)
            def _(i):
                h = pltpu.bitcast(jnp.concatenate(
                    [hc_s[2 * NP + a, words(i), :] for a in range(M // D)], axis=1), BF16)
                q = jnp.dot(h, weight(wq_v), preferred_element_type=F32) * qscale
                s = lax.dot_general(q.astype(BF16), _ld(k_s, (hd,), 0, S), NT,
                                    preferred_element_type=F32)
                s = jnp.where(lax.broadcasted_iota(jnp.int32, (T, S), 1)
                              <= i * T + lax.broadcasted_iota(jnp.int32, (T, S), 0), s, MASK)
                p = jnp.exp2(s - jnp.max(s, axis=1, keepdims=True))
                o = jnp.dot(p.astype(BF16), _ld(v_s, (0,), 0, S), preferred_element_type=F32)
                o = o * _recip(jnp.sum(p, axis=1, keepdims=True))
                hc_s[hd, words(i), :] = pltpu.bitcast(o.astype(BF16), U32)

    osem = sems.at[len(groups) + 1]
    lane = lax.broadcasted_iota(jnp.int32, (8, T), 1)
    sub = lax.broadcasted_iota(jnp.int32, (8, T), 0)
    ibits = (S - 1).bit_length()
    imask = (1 << ibits) - 1

    def sort_key(r, tok):
        u = lax.shift_right_logical(lax.bitcast_convert_type(r, jnp.int32), 16)
        u = jnp.where(u >= 0x8000, 0xFFFF - u, u + 0x8000)
        u = jnp.where(r == 0.0, 0x8000, u)
        u = jnp.where(r != r, 0, u)
        return lax.bitcast_convert_type(KEY_BASE + imask - tok + (u << ibits), F32)

    def merge_top(best, cols):
        new = jnp.zeros((8, T), F32)
        for a, col_ in enumerate(cols):
            new = jnp.where(lane == 8 * a + sub, col_, new)
        top = jnp.zeros((8, T), F32)
        for row in (new, jnp.where(lane == sub, best, 0.0)):
            row = jnp.max(row, axis=0, keepdims=True)
            above = [jnp.where(col_ > row, 1.0, 0.0) for col_ in cols + [best]]
            while len(above) > 1:
                above = [sum(above[a + 1:a + 2], above[a]) for a in range(0, len(above), 2)]
            rank = jnp.sum(above[0], axis=0, keepdims=True)
            top = jnp.where(rank == sub.astype(F32), row, top)
        return jnp.broadcast_to(jnp.max(top, axis=1, keepdims=True), (8, T))

    def oproj(lo, hi):
        for i in range(lo, hi):
            x1_s[i * T:(i + 1) * T, :] = jnp.dot(
                ld_wide(0, 2 * NP, i), wo_v[...], preferred_element_type=F32)

    def finalize(lo, hi, best):
        w_r = wr_v[...].astype(F32).reshape(1, M)
        for i in range(lo, hi):
            rs = slice(i * T, (i + 1) * T)
            x1 = _rb(x_v[rs, :].astype(F32) + mod_s[2:3, :] * x1_s[rs, :])
            mean, _, var = _moments(x1)
            rstd = 1.0 / _rb(jnp.sqrt(_rb(_rb(var) + EPS)))
            h2 = _rb(_rb(x1 - _rb(mean)) * rstd)
            h2 = _rb(_rb(h2 * mod_s[4:5, :]) + mod_s[3:4, :])
            out_s[rs, :] = (x1 + mod_s[5:6, :] * h2).astype(BF16)
            x1_s[rs, :] = x1
            h2_s[rs, :] = h2
            r = jnp.broadcast_to(_rb(jnp.sum(h2 * w_r, axis=1, keepdims=True)), (T, T))
            best = merge_top(best, [sort_key(r[a:a + 8], i * T + a + sub)
                                    for a in range(0, T, 8)])
        return best

    cuts = (0, 8, 13, 15, nb)
    out_cp = [pltpu.make_async_copy(out_s.at[pl.ds(lo * T, (hi - lo) * T)],
                                    out_hbm.at[pl.ds(lo * T, (hi - lo) * T)], osem)
              for lo, hi in zip(cuts, cuts[1:])]
    wait(copies(5))
    oproj(cuts[0], cuts[1])
    wgt_s[...] = wg_v[...].T
    wut_s[...] = wu_v[...].T
    best = jnp.zeros((8, T), F32)
    for n in range(1, len(cuts) - 1):
        wait(copies(5 + n))
        if n > 1:
            out_cp[n - 2].start()
        oproj(cuts[n], cuts[n + 1])
        best = finalize(cuts[n - 1], cuts[n], best)
    out_cp[-2].start()
    best = finalize(cuts[-2], cuts[-1], best)
    out_cp[-1].start()

    bi = lax.bitcast_convert_type(best, jnp.int32) - KEY_BASE
    u = bi >> ibits
    u = jnp.where(u >= 0x8000, u - 0x8000, 0xFFFF - u)
    r_sel = lax.bitcast_convert_type(u << 16, F32)[:, 0:1]
    tok = imask - (bi & imask)
    idx = [tok[k, 0] for k in range(TOPK)]

    xs = jnp.concatenate([x1_s[pl.ds(i, 1), :] for i in idx], axis=0)
    hs = jnp.concatenate([h2_s[pl.ds(i, 1), :] for i in idx], axis=0)
    hb = hs.astype(BF16)
    g = _rb(jnp.dot(hb, wgt_s[...], preferred_element_type=F32))
    up = _rb(jnp.dot(hb, wut_s[...], preferred_element_type=F32))
    a = (_rb(g * _sigmoid(g)) * up).astype(BF16)
    y = _rb(jnp.dot(a, wd_v[...], preferred_element_type=F32))
    y = _rb(y * _sigmoid(r_sel))
    new = _rb(xs + mod_s[5:6, :] * _rb(hs + y))

    wait(out_cp)
    row16 = lax.broadcasted_iota(jnp.int32, (16, M), 0)
    base = [pl.multiple_of(i & ~15, 16) for i in idx]
    for k in range(TOPK):
        old = out_s[pl.ds(base[k], 16), :].astype(F32)
        out_s[pl.ds(base[k], 16), :] = jnp.where(
            row16 == idx[k] - base[k], new[k:k + 1, :], old).astype(BF16)
    first = []
    for k in range(TOPK):
        f = True
        for j in range(k):
            f = jnp.logical_and(f, base[j] != base[k])
        first.append(f)
    patch = [pltpu.make_async_copy(out_s.at[pl.ds(base[k], 16)],
                                   out_hbm.at[pl.ds(base[k], 16)], osem)
             for k in range(TOPK)]
    for k in range(TOPK):
        pl.when(first[k])(patch[k].start)
    for k in range(TOPK):
        pl.when(first[k])(patch[k].wait)


@jax.jit
def pallas_adaLN_cond__compressed_kv_cla__moe_arch_mod__prompt_kernel(
    A_x: jax.Array,
    A_c_kv: jax.Array,
    A_w_q: jax.Array,
    A_w_uk: jax.Array,
    A_w_uv: jax.Array,
    A_w_o: jax.Array,
    B_x: jax.Array,
    B_w_r: jax.Array,
    B_w_gate: jax.Array,
    B_w_up: jax.Array,
    B_w_down: jax.Array,
    c: jax.Array,
    w_mod: jax.Array,
):
    del B_x
    B, S, M = A_x.shape
    C = A_c_kv.shape[2]
    _, H, D = A_w_q.shape
    F = B_w_gate.shape[1]
    NP = H // 2
    assert B == 1 and A_c_kv.shape[1] == S and (S, D, NP) == (2048, T, 16)
    vm = pltpu.VMEM
    out = pl.pallas_call(
        _kernel,
        out_shape=jax.ShapeDtypeStruct((S, M), A_x.dtype),
        in_specs=[pl.BlockSpec(memory_space=pltpu.HBM)] * 12,
        out_specs=pl.BlockSpec(memory_space=pltpu.HBM),
        scratch_shapes=[
            vm((S, M), BF16), vm((S, C), BF16), vm((NP, M, D), U32),
            vm((NP, C, D), U32), vm((NP, C, D), U32), vm((H * D, M), BF16),
            vm((M, 6 * M), BF16),
            vm((H, S // 2, D), U32), vm((2, S // 2, D), U32),
            vm((H + M // D, S // 2, D), U32), vm((S, M), F32), vm((S, M), F32), vm((S, M), BF16),
            vm((F, M), BF16), vm((F, M), BF16), vm((F, M), BF16),
            vm((M, F), BF16), vm((M, F), BF16),
            vm((8, M), F32), vm((M,), BF16), vm((1, M), BF16),
            pltpu.SemaphoreType.DMA((11,)),
        ],
        compiler_params=pltpu.CompilerParams(
            vmem_limit_bytes=110 * 2 ** 20, disable_bounds_checks=True,
            flags={"XLA_TPU_EVENLY_DISTRIBUTE_CRITICAL_NODES": True}),
        name="adaln_cla_moe",
    )(A_x.reshape(S, M), A_c_kv.reshape(S, C), A_w_q.reshape(M, NP, 2, D),
      A_w_uk.reshape(C, NP, 2, D), A_w_uv.reshape(C, NP, 2, D),
      A_w_o.reshape(H * D, M), B_w_r, B_w_gate.T, B_w_up.T, B_w_down, c, w_mod)
    return out.reshape(B, S, M)
```
